```python
import jax
import jax.numpy as jnp

def _softmax(x, axis=-1):
    return jax.nn.softmax(x, axis=axis)

def _gelu(x):
    return jax.nn.gelu(x, approximate=True)

def _silu(x):
    return jax.nn.silu(x)

def _sigmoid(x):
    return jax.nn.sigmoid(x)

def _layernorm(x, axis=-1, eps=1e-05):
    m = jnp.mean(x, axis=axis, keepdims=True)
    v = jnp.var(x, axis=axis, keepdims=True)
    return (x - m) / jnp.sqrt(v + eps)

def _scatter_add(tgt, idx, src, axis=0):
    return tgt.at[idx].add(src)

def _segment_sum(src, seg, n):
    return jax.ops.segment_sum(src, seg, n)

class _Rng:

    def __init__(self, key):
        self._k = key

    def _next(self):
        self._k, sub = jax.random.split(self._k)
        return sub

    def normal(self, shape):
        return jax.random.normal(self._next(), shape, dtype=jnp.bfloat16)

    def randint(self, lo, hi, shape):
        return jax.random.randint(self._next(), shape, lo, hi, dtype=jnp.int32)

    def uniform(self, shape, lo=0.0, hi=1.0):
        return jax.random.uniform(self._next(), shape, jnp.bfloat16, lo, hi)

    def permutation(self, n):
        return jax.random.permutation(self._next(), n)
kernel_name = 'concat_heads__sliding_local_dilated__memory_aug_recurrent_mem_tr__prompt'

def setup_inputs():
    _rng = _Rng(jax.random.key(int.from_bytes(__import__("os").urandom(4), "little")))
    _w = lambda a: (lambda t: t.astype(jnp.bfloat16) if jnp.issubdtype(t.dtype, jnp.floating) else t)(jnp.asarray(a))

    def _A_setup():
        B, S, D = (1, 2048, 640)
        return {'x': _w((lambda *s: _rng.normal(s) * 0.05)(B, S, D)), 'wqkv': _w((lambda *s: _rng.normal(s) * 0.05)(D, 3 * D)), 'wo': _w((lambda *s: _rng.normal(s) * 0.05)(D, D))}
    _A_in = _A_setup()

    def _B_setup():
        B, S, Dm = (1, 2048, 640)
        H, Dh = (32, 192)
        M, seg = (8, 32)
        seg = min(seg, S)
        S = S // seg * seg
        return {'x': _w((lambda *s: _rng.normal(s) * 0.05)(B, S, Dm)), 'mem0': _w((lambda *s: _rng.normal(s) * 0.05)(B, M, Dm)), 'Wq': _w((lambda *s: _rng.normal(s) * 0.05)(Dm, H, Dh) * Dm ** (-0.5)), 'Wk': _w((lambda *s: _rng.normal(s) * 0.05)(Dm, H, Dh) * Dm ** (-0.5)), 'Wv': _w((lambda *s: _rng.normal(s) * 0.05)(Dm, H, Dh) * Dm ** (-0.5)), 'Wo': _w((lambda *s: _rng.normal(s) * 0.05)(H, Dh, Dm) * (H * Dh) ** (-0.5)), 'seg_len': seg}
    _B_in = _B_setup()
    return {'A_x': _A_in['x'], 'A_wqkv': _A_in['wqkv'], 'A_wo': _A_in['wo'], 'B_x': _B_in['x'], 'B_mem0': _B_in['mem0'], 'B_Wq': _B_in['Wq'], 'B_Wk': _B_in['Wk'], 'B_Wv': _B_in['Wv'], 'B_Wo': _B_in['Wo'], 'B_seg_len': _B_in['seg_len']}

def reference(A_x, A_wqkv, A_wo, B_x, B_mem0, B_Wq, B_Wk, B_Wv, B_Wo, B_seg_len):

    def _A_ref(x, wqkv, wo):
        B, S, D = x.shape
        H = 32
        Dh = D // H
        W, dil = (8, 2)
        qkv = (lambda x, *d: x.transpose(*d))((x @ wqkv).reshape(B, S, 3, H, Dh), 2, 0, 3, 1, 4)
        q, k, v = (qkv[0], qkv[1], qkv[2])
        scale = Dh ** (-0.5)
        pos = jnp.arange(S)
        off = jnp.arange(W) * dil
        idx = pos[:, None] - off[None, :]
        mask = idx >= 0
        idx_c = jnp.where(mask, idx, 0).reshape(-1)
        kg = k[:, :, idx_c, :].reshape(B, H, S, W, Dh)
        vg = v[:, :, idx_c, :].reshape(B, H, S, W, Dh)
        logits = jnp.einsum('bhsd,bhswd->bhsw', q, kg) * scale
        logits = jnp.where(mask[None, None, :, :], logits, -1000000000.0)
        attn = _softmax(logits, axis=-1)
        o = jnp.einsum('bhsw,bhswd->bhsd', attn, vg)
        return (lambda x, *d: x.transpose(*d))(o, 0, 2, 1, 3).reshape(B, S, D) @ wo

    def _B_ref(x, mem0, Wq, Wk, Wv, Wo, seg_len):
        B, S, Dm = x.shape
        H, Dh = (Wq.shape[1], Wq.shape[2])
        M = mem0.shape[1]
        scale = Dh ** (-0.5)
        n_seg = S // seg_len
        L = M + seg_len
        idx = jnp.arange(L)
        mask = (idx[:, None] < M) | (idx[:, None] >= idx[None, :])
        mem = mem0
        outs = []
        for s in range(n_seg):
            xs = x[:, s * seg_len:(s + 1) * seg_len, :].copy()
            h = jnp.concatenate([mem, xs], axis=1)
            q = jnp.einsum('btd,dhe->bhte', h, Wq)
            k = jnp.einsum('btd,dhe->bhte', h, Wk)
            v = jnp.einsum('btd,dhe->bhte', h, Wv)
            scores = jnp.einsum('bhqe,bhke->bhqk', q, k) * scale
            scores = jnp.where(mask[None, None], scores, -1000000000.0)
            p = _softmax(scores, axis=-1)
            o = jnp.einsum('bhqk,bhke->bhqe', p, v)
            o = jnp.einsum('bhte,hed->btd', o, Wo)
            mem = o[:, :M, :].copy()
            outs.append(o[:, M:, :])
        return jnp.concatenate(outs, axis=1)
    a = _A_ref(A_x, A_wqkv, A_wo)
    b = _B_ref(B_x, B_mem0, B_Wq, B_Wk, B_Wv, B_Wo, B_seg_len)
    return jnp.concatenate([a, b], axis=-1)
```

```python
import jax
import jax.numpy as jnp
import numpy as np
from jax import lax
import jax.experimental.pallas as pl
import jax.experimental.pallas.tpu as pltpu

F32 = jnp.float32
BF16 = jnp.bfloat16
LANES = 128
NEG = -1000000000.0

A_HEADS = 32
A_WINDOW = 8
A_DILATION = 2
A_HALO = 16
A_CHUNK = 256
A_ROWS = 16


def _dot(a, b):
    return lax.dot_general(a, b, (((1,), (0,)), ((), ())), preferred_element_type=F32)


def _dot_nt(a, b):
    return lax.dot_general(a, b, (((1,), (1,)), ((), ())), preferred_element_type=F32)


def _pack(w):
    return pltpu.bitcast(w, jnp.int32)


def _unpack(w):
    return pltpu.bitcast(w, BF16)


def _make_kernel(S, D, H, Dh, M, seg):
    n_seg = S // seg
    L = M + seg
    n_pair = H // 2
    PW = 2 * Dh
    n_tile = D // LANES
    n_chunk = S // A_CHUNK
    pairs_per_chunk = n_pair // n_chunk
    a_dh = D // A_HEADS
    a_scale = float(a_dh) ** -0.5
    b_scale = float(Dh) ** -0.5

    def kernel(xa_hbm, wqkv_hbm, woa_hbm, xb_hbm, mem0_hbm, wqt_hbm, wkt_hbm, wvt_hbm, wob_hbm,
               out_hbm,
               xa_v, wqkv_v, woa_v, xb_v, mem0_v, wt_v, wob_v,
               wa_p, woa_p, q_s, k_s, v_s, oa_s, outa_v,
               w_p, wo_p, h_s, o_s, outb_v,
               sem_wa, sem_xa, sem_w, sem_wo, sem_xb, sem_out):
        def wa_copies():
            cps = [pltpu.make_async_copy(wqkv_hbm.at[:, pl.ds(t * D, D)], wqkv_v.at[t], sem_wa.at[t])
                   for t in range(3)]
            return cps + [pltpu.make_async_copy(woa_hbm, woa_v, sem_wa.at[3])]

        def xa_copy(c):
            rows = pl.ds(c * A_CHUNK, A_CHUNK)
            return pltpu.make_async_copy(xa_hbm.at[rows], xa_v.at[rows], sem_xa.at[c])

        def w_copy(t, c):
            rows = pl.ds(c * pairs_per_chunk * PW, pairs_per_chunk * PW)
            src = (wkt_hbm, wqt_hbm, wvt_hbm)[t]
            return pltpu.make_async_copy(src.at[rows], wt_v.at[t, rows], sem_w.at[t, c])

        wo_copy = pltpu.make_async_copy(wob_hbm, wob_v, sem_wo)
        xb_copy = pltpu.make_async_copy(xb_hbm, xb_v, sem_xb.at[0])
        mem_copy = pltpu.make_async_copy(mem0_hbm, mem0_v, sem_xb.at[1])

        for cp in wa_copies():
            cp.start()
        for c in range(n_chunk):
            xa_copy(c).start()
            for t in range(3):
                w_copy(t, c).start()
        wo_copy.start()
        mem_copy.start()
        xb_copy.start()

        r_i = lax.broadcasted_iota(jnp.int32, (D, D), 0)
        c_i = lax.broadcasted_iota(jnp.int32, (D, D), 1)
        perm = jnp.where(r_i == (c_i % A_HEADS) * a_dh + c_i // A_HEADS, 1.0, 0.0).astype(BF16)
        perm_t = jnp.where(c_i == (r_i % A_HEADS) * a_dh + r_i // A_HEADS, 1.0, 0.0).astype(BF16)
        cps = wa_copies()
        for t in range(3):
            cps[t].wait()
            wa_p[t] = _pack(_dot(wqkv_v[t], perm).astype(BF16))
        cps[3].wait()
        woa_p[...] = _pack(_dot(perm_t, woa_v[...]).astype(BF16))

        def a_chunk(c, first):
            r0 = c * A_CHUNK
            if not first:
                r0 = pl.multiple_of(r0, A_CHUNK)
            xa_copy(c).wait()
            for t in range(3):
                w_copy(t, c).wait()
            x = xa_v[pl.ds(r0, A_CHUNK), :]
            if not first:
                for j in range(n_tile):
                    k_s[j, 0:A_HALO, :] = k_s[j, A_CHUNK:A_CHUNK + A_HALO, :]
                    v_s[j, 0:A_HALO, :] = v_s[j, A_CHUNK:A_CHUNK + A_HALO, :]
            k = _dot(x, _unpack(wa_p[1]))
            for j in range(n_tile):
                k_s[j, A_HALO:, :] = k[:, j * LANES:(j + 1) * LANES]
            q_s[...] = _dot(x, _unpack(wa_p[0]))
            v = _dot(x, _unpack(wa_p[2]))
            for j in range(n_tile):
                v_s[j, A_HALO:, :] = v[:, j * LANES:(j + 1) * LANES]
            if first:
                for j in range(n_tile):
                    k_s[j, 0:A_HALO, :] = jnp.broadcast_to(k_s[j, A_HALO:A_HALO + 1, :], (A_HALO, LANES))
                    v_s[j, 0:A_HALO, :] = jnp.broadcast_to(v_s[j, A_HALO:A_HALO + 1, :], (A_HALO, LANES))

            for i in range(pairs_per_chunk):
                p = c * pairs_per_chunk + i
                rows = p * PW
                if not first:
                    rows = pl.multiple_of(rows, PW)
                for t in range(3):
                    w_p[p, t] = _pack(wt_v[t, pl.ds(rows, PW), :].T)

            for b in range(A_CHUNK // A_ROWS):
                b0 = b * A_ROWS
                q = [q_s[b0:b0 + A_ROWS, j * LANES:(j + 1) * LANES] for j in range(n_tile)]
                logits = []
                for w in range(A_WINDOW):
                    a0 = A_HALO + b0 - w * A_DILATION
                    t = q[0] * k_s[0, a0:a0 + A_ROWS, :]
                    for j in range(1, n_tile):
                        t = t + q[j] * k_s[j, a0:a0 + A_ROWS, :]
                    t = t + pltpu.roll(t, 64, 1)
                    t = t + pltpu.roll(t, 32, 1)
                    t = t * a_scale
                    if first and b0 < w * A_DILATION:
                        pos = b0 + lax.broadcasted_iota(jnp.int32, (A_ROWS, LANES), 0)
                        t = jnp.where(pos >= w * A_DILATION, t, NEG)
                    logits.append(t)
                mx = logits[0]
                for t in logits[1:]:
                    mx = jnp.maximum(mx, t)
                e = [jnp.exp(t - mx) for t in logits]
                den = e[0]
                for t in e[1:]:
                    den = den + t
                inv = 1.0 / den
                for j in range(n_tile):
                    acc = e[0] * v_s[j, A_HALO + b0:A_HALO + b0 + A_ROWS, :]
                    for w in range(1, A_WINDOW):
                        a0 = A_HALO + b0 - w * A_DILATION
                        acc = acc + e[w] * v_s[j, a0:a0 + A_ROWS, :]
                    oa_s[b0:b0 + A_ROWS, j * LANES:(j + 1) * LANES] = acc * inv
            half = A_CHUNK // 2
            for i in range(2):
                y = _dot(oa_s[i * half:(i + 1) * half, :], _unpack(woa_p[...]))
                outa_v[pl.ds(r0 + i * half, half), :] = y.astype(BF16)

        a_chunk(0, True)

        def a_body(c, carry):
            a_chunk(c, False)
            return carry

        lax.fori_loop(1, n_chunk, a_body, 0)

        outa_copy = pltpu.make_async_copy(outa_v, out_hbm.at[:, pl.ds(0, D)], sem_out.at[0])

        wo_copy.wait()

        def wo_body(p, carry):
            wo_p[p] = _pack(wob_v[pl.ds(pl.multiple_of(p * PW, PW), PW), :])
            return carry

        lax.fori_loop(0, n_pair, wo_body, 0)
        mem_copy.wait()
        xb_copy.wait()
        outa_copy.start()
        h_s[0:M, :] = mem0_v[...].astype(F32)

        row = lax.broadcasted_iota(jnp.int32, (L, LANES), 0)
        lane = lax.broadcasted_iota(jnp.int32, (L, LANES), 1)
        key = jnp.where(lane < L, lane, lane - L)
        visible = (row < M) | (row >= key)
        in0 = lane < L
        in1 = (lane >= L) & (lane < 2 * L)
        fill0 = jnp.where(in0, NEG, -jnp.inf).astype(F32)
        fill1 = jnp.where(in1, NEG, -jnp.inf).astype(F32)
        split = Dh - LANES
        lo = lane < split

        def block_diag(t):
            z = jnp.zeros((L, LANES), F32)
            mid = t[:, LANES:2 * LANES]
            top = jnp.concatenate([t[:, :LANES], jnp.where(lo, mid, 0.0), z], axis=1)
            bot = jnp.concatenate([z, jnp.where(lo, 0.0, mid), t[:, 2 * LANES:]], axis=1)
            pad = jnp.zeros((LANES - 2 * L, PW), F32)
            return jnp.concatenate([top, bot, pad], axis=0).astype(BF16)

        def softmax2(s):
            s = s * b_scale
            s0 = jnp.where(visible & in0, s, fill0)
            s1 = jnp.where(visible & in1, s, fill1)
            m0 = jnp.max(s0, axis=1, keepdims=True)
            m1 = jnp.max(s1, axis=1, keepdims=True)
            e = jnp.exp(jnp.where(in0, s0 - m0, s1 - m1))
            d0 = jnp.sum(jnp.where(in0, e, 0.0), axis=1, keepdims=True)
            d1 = jnp.sum(jnp.where(in0, 0.0, e), axis=1, keepdims=True)
            return e / jnp.where(in0, d0, d1)

        def outb_copy(r0):
            return pltpu.make_async_copy(
                outb_v.at[pl.ds(r0, seg)], out_hbm.at[pl.ds(r0, seg), pl.ds(D, D)], sem_out.at[1])

        def out_proj(p0, p1):
            w = _unpack(wo_p[p0:p1].reshape((p1 - p0) * PW // 2, D))
            return _dot(o_s[:, p0 * PW:p1 * PW], w)

        def seg_body(s, carry):
            r0 = pl.multiple_of(s * seg, seg)
            h_s[M:, :] = xb_v[pl.ds(r0, seg), :].astype(F32)
            prob = None
            vbd = None
            acc = None
            for p in range(n_pair):
                h = h_s[...]
                k = _dot(h, _unpack(w_p[p, 0]))
                q = _dot(h, _unpack(w_p[p, 1]))
                v = _dot(h, _unpack(w_p[p, 2]))
                if p > 0:
                    o_s[:, (p - 1) * PW:p * PW] = _dot(prob, vbd)
                if p == n_pair - 1:
                    acc = out_proj(0, 4)
                prob = softmax2(_dot_nt(q, block_diag(k)))
                vbd = block_diag(v)
            acc = acc + out_proj(4, 12)
            o_s[:, (n_pair - 1) * PW:] = _dot(prob, vbd)
            acc = acc + out_proj(12, 15)
            acc = acc + out_proj(15, 16)
            h_s[0:M, :] = acc[0:M]
            outb_v[pl.ds(r0, seg), :] = acc[M:].astype(BF16)
            outb_copy(r0).start()
            return carry

        lax.fori_loop(0, n_seg, seg_body, 0)

        outa_copy.wait()
        pltpu.make_async_copy(outb_v, outb_v, sem_out.at[1]).wait()

    scratch = [
        pltpu.VMEM((S, D), BF16),
        pltpu.VMEM((3, D, D), BF16),
        pltpu.VMEM((D, D), BF16),
        pltpu.VMEM((S, D), BF16),
        pltpu.VMEM((M, D), BF16),
        pltpu.VMEM((3, H * Dh, D), BF16),
        pltpu.VMEM((H * Dh, D), BF16),
        pltpu.VMEM((3, D // 2, D), jnp.int32),
        pltpu.VMEM((D // 2, D), jnp.int32),
        pltpu.VMEM((A_CHUNK, D), F32),
        pltpu.VMEM((n_tile, A_HALO + A_CHUNK, LANES), F32),
        pltpu.VMEM((n_tile, A_HALO + A_CHUNK, LANES), F32),
        pltpu.VMEM((A_CHUNK, D), F32),
        pltpu.VMEM((S, D), BF16),
        pltpu.VMEM((n_pair, 3, D // 2, PW), jnp.int32),
        pltpu.VMEM((n_pair, PW // 2, D), jnp.int32),
        pltpu.VMEM((L, D), F32),
        pltpu.VMEM((L, H * Dh), F32),
        pltpu.VMEM((S, D), BF16),
        pltpu.SemaphoreType.DMA((4,)),
        pltpu.SemaphoreType.DMA((n_chunk,)),
        pltpu.SemaphoreType.DMA((3, n_chunk)),
        pltpu.SemaphoreType.DMA,
        pltpu.SemaphoreType.DMA((2,)),
        pltpu.SemaphoreType.DMA((2,)),
    ]
    return kernel, scratch


def pallas_concat_heads__sliding_local_dilated__memory_aug_recurrent_mem_tr__prompt_kernel(
    A_x, A_wqkv, A_wo, B_x, B_mem0, B_Wq, B_Wk, B_Wv, B_Wo, B_seg_len,
):
    _, S, D = A_x.shape
    _, H, Dh = B_Wq.shape
    M = B_mem0.shape[1]
    seg = int(B_seg_len)
    kernel, scratch = _make_kernel(S, D, H, Dh, M, seg)

    def rows_first(w):
        return jnp.transpose(w, (1, 2, 0)).reshape(H * Dh, D)

    out = pl.pallas_call(
        kernel,
        out_shape=jax.ShapeDtypeStruct((S, 2 * D), BF16),
        in_specs=[pl.BlockSpec(memory_space=pl.ANY)] * 9,
        out_specs=pl.BlockSpec(memory_space=pl.ANY),
        scratch_shapes=scratch,
        compiler_params=pltpu.CompilerParams(vmem_limit_bytes=110 * 2**20),
    )(
        A_x.reshape(S, D), A_wqkv, A_wo, B_x.reshape(S, D), B_mem0.reshape(M, D),
        rows_first(B_Wq), rows_first(B_Wk), rows_first(B_Wv), B_Wo.reshape(H * Dh, D),
    )
    return out.reshape(1, S, 2 * D)
```

```python
import jax
import jax.numpy as jnp
import numpy as np
from jax import lax
import jax.experimental.pallas as pl
import jax.experimental.pallas.tpu as pltpu

F32 = jnp.float32
BF16 = jnp.bfloat16
LANES = 128
NEG = -1000000000.0
LOG2E = float(np.log2(np.e))

A_HEADS = 32
A_WINDOW = 8
A_DILATION = 2
A_HALO = 16
A_CHUNK = 256
A_UNIT = 128
A_ROWS = 16
WO_CHUNKS = 8
UNROLL = 1
XB_HEAD = 32 * (UNROLL + 1)
HEAD_PAIRS = 12


def _dot(a, b):
    return lax.dot_general(a, b, (((1,), (0,)), ((), ())), preferred_element_type=F32)


def _dot_nt(a, b):
    return lax.dot_general(a, b, (((1,), (1,)), ((), ())), preferred_element_type=F32)


def _pack(w):
    return pltpu.bitcast(w, jnp.int32)


def _unpack(w):
    return pltpu.bitcast(w, BF16)


def _make_kernel(S, D, H, Dh, M, seg):
    n_seg = S // seg
    L = M + seg
    n_pair = H // 2
    PW = 2 * Dh
    n_tile = D // LANES
    n_chunk = S // A_CHUNK
    pairs_per_chunk = n_pair // n_chunk
    pairs_per_wo = n_pair // WO_CHUNKS
    a_dh = D // A_HEADS
    a_scale = float(a_dh) ** -0.5
    b_scale = float(Dh) ** -0.5

    def kernel(xa_hbm, wqkv_hbm, woa_hbm, xb_hbm, mem0_hbm, wqt_hbm, wkt_hbm, wvt_hbm, wob_hbm,
               out_hbm,
               xa_v, wqkv_v, woa_v, xb_v, mem0_v, wt_v, wob_v,
               perm_s, wa_p, q_s, k_s, v_s, oa_s, outa_v,
               w_p, wo_p, h_s, o_s, acc_s, outb_v,
               sem_in, sem_out):
        def wa_copy(t):
            if t == 3:
                return pltpu.make_async_copy(woa_hbm, woa_v, sem_in.at[3])
            return pltpu.make_async_copy(wqkv_hbm.at[:, pl.ds(t * D, D)], wqkv_v.at[t], sem_in.at[t])

        def xa_copy(c):
            rows = pl.ds(c * A_CHUNK, A_CHUNK)
            return pltpu.make_async_copy(xa_hbm.at[rows], xa_v.at[rows], sem_in.at[6 + WO_CHUNKS + 4 * c])

        def w_copy(t, c):
            rows = pl.ds(c * pairs_per_chunk * PW, pairs_per_chunk * PW)
            src = (wkt_hbm, wqt_hbm, wvt_hbm)[t]
            return pltpu.make_async_copy(src.at[rows], wt_v.at[t, rows], sem_in.at[7 + WO_CHUNKS + 4 * c + t])

        def wo_copy(c):
            rows = pl.ds(c * pairs_per_wo * PW, pairs_per_wo * PW)
            return pltpu.make_async_copy(wob_hbm.at[rows], wob_v.at[rows], sem_in.at[6 + c])

        xb_head = pltpu.make_async_copy(xb_hbm.at[pl.ds(0, XB_HEAD)], xb_v.at[pl.ds(0, XB_HEAD)], sem_in.at[4])
        xb_rest = pltpu.make_async_copy(
            xb_hbm.at[pl.ds(XB_HEAD, S - XB_HEAD)], xb_v.at[pl.ds(XB_HEAD, S - XB_HEAD)], sem_in.at[6 + WO_CHUNKS + 4 * n_chunk])
        mem_copy = pltpu.make_async_copy(mem0_hbm, mem0_v, sem_in.at[5])

        for t in range(4):
            wa_copy(t).start()
        xa_copy(0).start()
        for c in range(n_chunk):
            for t in range(3):
                w_copy(t, c).start()
            if c + 1 < n_chunk:
                xa_copy(c + 1).start()
        mem_copy.start()
        xb_head.start()
        for c in range(WO_CHUNKS):
            wo_copy(c).start()
        xb_rest.start()

        def store_reordered(t, w):
            w = _pack(w)
            for j in range(n_tile):
                perm_s[j] = w[:, j * LANES:(j + 1) * LANES]
            for dd in range(a_dh // 2):
                for j in range(n_tile):
                    u = perm_s[j, pl.ds(dd, A_HEADS, stride=a_dh // 2), :]
                    even = pltpu.bitcast(u << 16, F32)
                    odd = pltpu.bitcast(u & jnp.int32(-65536), F32)
                    both = jnp.concatenate([even, odd], axis=0).astype(BF16)
                    wa_p[t, dd * A_HEADS:(dd + 1) * A_HEADS, j * LANES:(j + 1) * LANES] = _pack(both)

        for t in range(3):
            wa_copy(t).wait()
            store_reordered(t, wqkv_v[t].T)
        wa_copy(3).wait()
        store_reordered(3, woa_v[...])
        for j in range(n_tile):
            k_s[j, A_CHUNK:, :] = jnp.zeros((A_HALO, LANES), F32)
            v_s[j, A_CHUNK:, :] = jnp.zeros((A_HALO, LANES), F32)

        def a_attend(b0, r0):
            q = [q_s[b0:b0 + A_ROWS, j * LANES:(j + 1) * LANES] for j in range(n_tile)]
            logits = []
            for w in range(A_WINDOW):
                a0 = A_HALO + b0 - w * A_DILATION
                t = q[0] * k_s[0, a0:a0 + A_ROWS, :]
                for j in range(1, n_tile):
                    t = t + q[j] * k_s[j, a0:a0 + A_ROWS, :]
                t = t + pltpu.roll(t, 64, 1)
                t = t + pltpu.roll(t, 32, 1)
                if b0 < w * A_DILATION:
                    pos = r0 + b0 + lax.broadcasted_iota(jnp.int32, (A_ROWS, LANES), 0)
                    t = jnp.where(pos >= w * A_DILATION, t, NEG * LOG2E)
                logits.append(t)
            mx = logits[0]
            for t in logits[1:]:
                mx = jnp.maximum(mx, t)
            e = [jnp.exp2(t - mx) for t in logits]
            den = e[0]
            for t in e[1:]:
                den = den + t
            inv = 1.0 / den
            for j in range(n_tile):
                acc = e[0] * v_s[j, A_HALO + b0:A_HALO + b0 + A_ROWS, :]
                for w in range(1, A_WINDOW):
                    a0 = A_HALO + b0 - w * A_DILATION
                    acc = acc + e[w] * v_s[j, a0:a0 + A_ROWS, :]
                oa_s[b0:b0 + A_ROWS, j * LANES:(j + 1) * LANES] = acc * inv

        def wait_weights(c):
            for t in range(3):
                w_copy(t, c).wait()

        def transpose_weights(c):
            for i in range(pairs_per_chunk):
                p = c * pairs_per_chunk + i
                rows = p * PW if isinstance(p, int) else pl.multiple_of(p * PW, PW)
                for t in range(3):
                    w_p[p, t] = _pack(wt_v[t, pl.ds(rows, PW), :].T)

        def a_body(c, carry):
            r0 = pl.multiple_of(c * A_CHUNK, A_CHUNK)
            xa_copy(c).wait()

            @pl.when(c > 0)
            def _():
                wait_weights(c - 1)

            transpose_weights(jnp.where(c == 0, n_chunk, c - 1))
            for j in range(n_tile):
                k_s[j, 0:A_HALO, :] = k_s[j, A_CHUNK:, :]
            v_tail = [v_s[j, A_CHUNK:, :] for j in range(n_tile)]
            for u0 in range(0, A_CHUNK, A_UNIT):
                x = xa_v[pl.ds(r0 + u0, A_UNIT), :]
                k = _dot_nt(x, _unpack(wa_p[1]))
                for j in range(n_tile):
                    k_s[j, A_HALO + u0:A_HALO + u0 + A_UNIT, :] = k[:, j * LANES:(j + 1) * LANES]
                q_s[u0:u0 + A_UNIT, :] = _dot_nt(x, _unpack(wa_p[0])) * (a_scale * LOG2E)
                v = _dot_nt(x, _unpack(wa_p[2]))
                for j in range(n_tile):
                    vj = v[:, j * LANES:(j + 1) * LANES]
                    v_s[j, A_HALO + u0:A_HALO + u0 + A_UNIT, :] = vj
                    if u0 == 0:
                        first = jnp.broadcast_to(vj[0:1], (A_HALO, LANES))
                        v_s[j, 0:A_HALO, :] = jnp.where(c == 0, first, v_tail[j])
                for b0 in range(u0, u0 + A_UNIT, A_ROWS):
                    a_attend(b0, r0)
            for u0 in range(0, A_CHUNK, A_UNIT):
                y = _dot(oa_s[u0:u0 + A_UNIT, :], _unpack(wa_p[3]))
                outa_v[pl.ds(r0 + u0, A_UNIT), :] = y.astype(BF16)
            return carry

        with jax.named_scope('A'):
            lax.fori_loop(0, n_chunk, a_body, 0)

        outa_copy = pltpu.make_async_copy(outa_v, out_hbm.at[:, pl.ds(0, D)], sem_out.at[0])

        row = lax.broadcasted_iota(jnp.int32, (L, LANES), 0)
        lane = lax.broadcasted_iota(jnp.int32, (L, LANES), 1)
        key = jnp.where(lane < L, lane, lane - L)
        visible = (row < M) | (row >= key)
        in0 = lane < L
        in1 = (lane >= L) & (lane < 2 * L)
        fill0 = jnp.where(in0, NEG * LOG2E, -jnp.inf).astype(F32)
        fill1 = jnp.where(in1, NEG * LOG2E, -jnp.inf).astype(F32)
        split = Dh - LANES
        lo = lane < split

        def block_diag(t):
            z = jnp.zeros((L, LANES), F32)
            mid = t[:, LANES:2 * LANES]
            top = jnp.concatenate([t[:, :LANES], jnp.where(lo, mid, 0.0), z], axis=1)
            bot = jnp.concatenate([z, jnp.where(lo, 0.0, mid), t[:, 2 * LANES:]], axis=1)
            pad = jnp.zeros((LANES - 2 * L, PW), F32)
            return jnp.concatenate([top, bot, pad], axis=0).astype(BF16)

        def softmax2(s):
            s = s * (b_scale * LOG2E)
            s0 = jnp.where(visible & in0, s, fill0)
            s1 = jnp.where(visible & in1, s, fill1)
            m0 = jnp.max(s0, axis=1, keepdims=True)
            m1 = jnp.max(s1, axis=1, keepdims=True)
            e = jnp.exp2(jnp.where(in0, s0 - m0, s1 - m1))
            d0 = jnp.sum(jnp.where(in0, e, 0.0), axis=1, keepdims=True)
            d1 = jnp.sum(jnp.where(in0, 0.0, e), axis=1, keepdims=True)
            return e / jnp.where(in0, d0, d1)

        def outb_copy(r0):
            return pltpu.make_async_copy(
                outb_v.at[pl.ds(r0, seg)], out_hbm.at[pl.ds(r0, seg), pl.ds(D, D)], sem_out.at[1])

        def out_proj(p0, p1):
            w = _unpack(wo_p[p0:p1].reshape((p1 - p0) * PW // 2, D))
            return _dot(o_s[:, p0 * PW:p1 * PW], w)

        def attend(r0, with_head):
            h_s[M:, :] = xb_v[pl.ds(r0, seg), :].astype(F32)
            prob = vbd = acc = None
            for p in range(n_pair):
                h = h_s[...]
                if p == 0:
                    c0 = D - LANES
                    k = _dot(h[:, c0:], _unpack(w_p[p, 0, c0 // 2:]))
                    q = _dot(h[:, c0:], _unpack(w_p[p, 1, c0 // 2:]))
                    k = k + _dot(h[:, :c0], _unpack(w_p[p, 0, :c0 // 2]))
                    q = q + _dot(h[:, :c0], _unpack(w_p[p, 1, :c0 // 2]))
                else:
                    k = _dot(h, _unpack(w_p[p, 0]))
                    q = _dot(h, _unpack(w_p[p, 1]))
                v = _dot(h, _unpack(w_p[p, 2]))
                if p > 0:
                    o_s[:, (p - 1) * PW:p * PW] = _dot(prob, vbd)
                if with_head and p == n_pair - 1:
                    acc = out_proj(0, 2)
                prob = softmax2(_dot_nt(q, block_diag(k)))
                vbd = block_diag(v)
            if with_head:
                acc = acc + out_proj(2, HEAD_PAIRS - 1)
            o_s[:, (n_pair - 1) * PW:] = _dot(prob, vbd)
            if with_head:
                acc_s[...] = acc + out_proj(HEAD_PAIRS - 1, HEAD_PAIRS)

        def finish(r0):
            acc = acc_s[...] + out_proj(HEAD_PAIRS, n_pair)
            h_s[0:M, :] = acc[0:M]
            outb_v[pl.ds(r0, seg), :] = acc[M:].astype(BF16)
            outb_copy(r0).start()

        with jax.named_scope('wait_xb'):
            mem_copy.wait()
            xb_head.wait()
            wait_weights(n_chunk - 1)
        transpose_weights(n_chunk - 1)
        h_s[0:M, :] = mem0_v[...].astype(F32)
        attend(0, False)

        acc_s[...] = jnp.zeros((L, D), F32)

        def repack_wo(c):
            wo_copy(c).wait()
            w = wob_v[pl.ds(pl.multiple_of(c * pairs_per_wo * PW, PW), pairs_per_wo * PW), :]
            wo_p[pl.ds(c * pairs_per_wo, pairs_per_wo)] = _pack(w).reshape(pairs_per_wo, PW // 2, D)
            return w

        def wo_head(c, carry):
            w = repack_wo(c)
            cols = pl.ds(pl.multiple_of(c * pairs_per_wo * PW, LANES), pairs_per_wo * PW)
            acc_s[...] += _dot(o_s[:, cols], w)
            return carry

        def wo_tail(c, carry):
            repack_wo(c)
            return carry

        with jax.named_scope('wo'):
            lax.fori_loop(0, HEAD_PAIRS // pairs_per_wo, wo_head, 0)
            lax.fori_loop(HEAD_PAIRS // pairs_per_wo, WO_CHUNKS, wo_tail, 0)
        outa_copy.start()

        def seg_body(i, carry):
            @pl.when(i == 1)
            def _():
                xb_rest.wait()

            for u in range(UNROLL):
                r0 = pl.multiple_of((i * UNROLL + u) * seg, seg)
                finish(r0)
                attend(pl.multiple_of(r0 + seg, seg), True)
            return carry

        with jax.named_scope('B'):
            lax.fori_loop(0, (n_seg - 1) // UNROLL, seg_body, 0)
        finish((n_seg - 1) * seg)

        outa_copy.wait()
        pltpu.make_async_copy(outb_v, outb_v, sem_out.at[1]).wait()

    scratch = [
        pltpu.VMEM((S, D), BF16),
        pltpu.VMEM((3, D, D), BF16),
        pltpu.VMEM((D, D), BF16),
        pltpu.VMEM((S, D), BF16),
        pltpu.VMEM((M, D), BF16),
        pltpu.VMEM((3, (n_pair + pairs_per_chunk) * PW, D), BF16),
        pltpu.VMEM((H * Dh, D), BF16),
        pltpu.VMEM((n_tile, D // 2, LANES), jnp.int32),
        pltpu.VMEM((4, D // 2, D), jnp.int32),
        pltpu.VMEM((A_CHUNK, D), F32),
        pltpu.VMEM((n_tile, A_HALO + A_CHUNK, LANES), F32),
        pltpu.VMEM((n_tile, A_HALO + A_CHUNK, LANES), F32),
        pltpu.VMEM((A_CHUNK, D), F32),
        pltpu.VMEM((S, D), BF16),
        pltpu.VMEM((n_pair + pairs_per_chunk, 3, D // 2, PW), jnp.int32),
        pltpu.VMEM((n_pair, PW // 2, D), jnp.int32),
        pltpu.VMEM((L, D), F32),
        pltpu.VMEM((L, H * Dh), F32),
        pltpu.VMEM((L, D), F32),
        pltpu.VMEM((S, D), BF16),
        pltpu.SemaphoreType.DMA((7 + WO_CHUNKS + 4 * n_chunk,)),
        pltpu.SemaphoreType.DMA((2,)),
    ]
    return kernel, scratch


def pallas_concat_heads__sliding_local_dilated__memory_aug_recurrent_mem_tr__prompt_kernel(
    A_x, A_wqkv, A_wo, B_x, B_mem0, B_Wq, B_Wk, B_Wv, B_Wo, B_seg_len,
):
    _, S, D = A_x.shape
    _, H, Dh = B_Wq.shape
    M = B_mem0.shape[1]
    seg = int(B_seg_len)
    kernel, scratch = _make_kernel(S, D, H, Dh, M, seg)

    def rows_first(w):
        return jnp.transpose(w, (1, 2, 0)).reshape(H * Dh, D)

    out = pl.pallas_call(
        kernel,
        out_shape=jax.ShapeDtypeStruct((S, 2 * D), BF16),
        in_specs=[pl.BlockSpec(memory_space=pl.ANY)] * 9,
        out_specs=pl.BlockSpec(memory_space=pl.ANY),
        scratch_shapes=scratch,
        compiler_params=pltpu.CompilerParams(vmem_limit_bytes=110 * 2**20),
    )(
        A_x.reshape(S, D), A_wqkv, A_wo, B_x.reshape(S, D), B_mem0.reshape(M, D),
        rows_first(B_Wq), rows_first(B_Wk), rows_first(B_Wv), B_Wo.reshape(H * Dh, D),
    )
    return out.reshape(1, S, 2 * D)
```

```python
import jax
import jax.numpy as jnp
import numpy as np
from jax import lax
import jax.experimental.pallas as pl
import jax.experimental.pallas.tpu as pltpu

F32 = jnp.float32
BF16 = jnp.bfloat16
LANES = 128
NEG = -1000000000.0
LOG2E = float(np.log2(np.e))

A_HEADS = 32
A_WINDOW = 8
A_DILATION = 2
A_HALO = 16
A_CHUNK = 256
A_UNIT = 128
A_ROWS = 16
WO_CHUNKS = 8
UNROLL = 3
XB_HEAD = 32 * (UNROLL + 1)
HEAD_PAIRS = 12


def _dot(a, b):
    return lax.dot_general(a, b, (((1,), (0,)), ((), ())), preferred_element_type=F32)


def _dot_nt(a, b):
    return lax.dot_general(a, b, (((1,), (1,)), ((), ())), preferred_element_type=F32)


def _pack(w):
    return pltpu.bitcast(w, jnp.int32)


def _unpack(w):
    return pltpu.bitcast(w, BF16)


def _make_kernel(S, D, H, Dh, M, seg):
    n_seg = S // seg
    L = M + seg
    n_pair = H // 2
    PW = 2 * Dh
    n_tile = D // LANES
    n_chunk = S // A_CHUNK
    per_step = -(-3 * n_pair // (n_chunk - 1))
    n_spare = per_step * n_chunk - 3 * n_pair
    pairs_per_wo = n_pair // WO_CHUNKS
    a_dh = D // A_HEADS
    a_scale = float(a_dh) ** -0.5
    b_scale = float(Dh) ** -0.5

    def kernel(xa_hbm, wqkv_hbm, woa_hbm, xb_hbm, mem0_hbm, wqt_hbm, wkt_hbm, wvt_hbm, wob_hbm,
               out_hbm,
               xa_v, wqkv_v, woa_v, xb_v, mem0_v, wt_v, wob_v,
               perm_s, wa_p, q_s, k_s, v_s, oa_s, outa_v,
               w_p, wo_p, h_s, o_s, acc_s, outb_v,
               sem_in, sem_out):
        def wa_copy(t):
            if t == 3:
                return pltpu.make_async_copy(woa_hbm, woa_v, sem_in.at[3])
            return pltpu.make_async_copy(wqkv_hbm.at[:, pl.ds(t * D, D)], wqkv_v.at[t], sem_in.at[t])

        def xa_copy(c):
            rows = pl.ds(c * A_CHUNK, A_CHUNK)
            return pltpu.make_async_copy(xa_hbm.at[rows], xa_v.at[rows], sem_in.at[7 + WO_CHUNKS + c])

        def w_start(n):
            src = (wkt_hbm, wqt_hbm, wvt_hbm)[n % 3]
            pltpu.make_async_copy(src.at[pl.ds(n // 3 * PW, PW)], wt_v.at[n + n_spare],
                                  sem_in.at[7 + WO_CHUNKS + n_chunk + (n + n_spare) // per_step]).start()

        def w_wait(c, n):
            blocks = wt_v.at[pl.ds(0, n)]
            pltpu.make_async_copy(blocks, blocks, sem_in.at[7 + WO_CHUNKS + n_chunk + c]).wait()

        def wo_copy(c):
            rows = pl.ds(c * pairs_per_wo * PW, pairs_per_wo * PW)
            return pltpu.make_async_copy(wob_hbm.at[rows], wob_v.at[rows], sem_in.at[6 + c])

        xb_head = pltpu.make_async_copy(xb_hbm.at[pl.ds(0, XB_HEAD)], xb_v.at[pl.ds(0, XB_HEAD)], sem_in.at[4])
        xb_rest = pltpu.make_async_copy(
            xb_hbm.at[pl.ds(XB_HEAD, S - XB_HEAD)], xb_v.at[pl.ds(XB_HEAD, S - XB_HEAD)], sem_in.at[6 + WO_CHUNKS])
        mem_copy = pltpu.make_async_copy(mem0_hbm, mem0_v, sem_in.at[5])

        for t in range(4):
            wa_copy(t).start()
        xa_copy(0).start()
        for c in range(1, n_chunk):
            xa_copy(c).start()
            for n in range(max(c * per_step - n_spare, 0), (c + 1) * per_step - n_spare):
                w_start(n)
        mem_copy.start()
        xb_head.start()
        for c in range(WO_CHUNKS):
            wo_copy(c).start()
        xb_rest.start()

        def store_reordered(t, w):
            w = _pack(w)
            for j in range(n_tile):
                perm_s[j] = w[:, j * LANES:(j + 1) * LANES]
            for dd in range(a_dh // 2):
                for j in range(n_tile):
                    u = perm_s[j, pl.ds(dd, A_HEADS, stride=a_dh // 2), :]
                    even = pltpu.bitcast(u << 16, F32)
                    odd = pltpu.bitcast(u & jnp.int32(-65536), F32)
                    both = jnp.concatenate([even, odd], axis=0).astype(BF16)
                    wa_p[t, dd * A_HEADS:(dd + 1) * A_HEADS, j * LANES:(j + 1) * LANES] = _pack(both)

        for t in range(3):
            wa_copy(t).wait()
            store_reordered(t, wqkv_v[t].T)
        wa_copy(3).wait()
        store_reordered(3, woa_v[...])
        for j in range(n_tile):
            k_s[j, A_CHUNK:, :] = jnp.zeros((A_HALO, LANES), F32)
            v_s[j, A_CHUNK:, :] = jnp.zeros((A_HALO, LANES), F32)

        def a_attend(b0, r0):
            q = [q_s[b0:b0 + A_ROWS, j * LANES:(j + 1) * LANES] for j in range(n_tile)]
            logits = []
            for w in range(A_WINDOW):
                a0 = A_HALO + b0 - w * A_DILATION
                t = q[0] * k_s[0, a0:a0 + A_ROWS, :]
                for j in range(1, n_tile):
                    t = t + q[j] * k_s[j, a0:a0 + A_ROWS, :]
                t = t + pltpu.roll(t, 64, 1)
                t = t + pltpu.roll(t, 32, 1)
                if b0 < w * A_DILATION:
                    pos = r0 + b0 + lax.broadcasted_iota(jnp.int32, (A_ROWS, LANES), 0)
                    t = jnp.where(pos >= w * A_DILATION, t, NEG * LOG2E)
                logits.append(t)
            mx = logits[0]
            for t in logits[1:]:
                mx = jnp.maximum(mx, t)
            e = [jnp.exp2(t - mx) for t in logits]
            den = e[0]
            for t in e[1:]:
                den = den + t
            inv = 1.0 / den
            for j in range(n_tile):
                acc = e[0] * v_s[j, A_HALO + b0:A_HALO + b0 + A_ROWS, :]
                for w in range(1, A_WINDOW):
                    a0 = A_HALO + b0 - w * A_DILATION
                    acc = acc + e[w] * v_s[j, a0:a0 + A_ROWS, :]
                oa_s[b0:b0 + A_ROWS, j * LANES:(j + 1) * LANES] = acc * inv

        def a_body(c, carry):
            r0 = pl.multiple_of(c * A_CHUNK, A_CHUNK)
            xa_copy(c).wait()

            @pl.when(c == 1)
            def _():
                w_wait(c, 2 * per_step - n_spare)

            @pl.when(c > 1)
            def _():
                w_wait(c, per_step)

            for i in range(per_step):
                w_p[c * per_step + i] = _pack(wt_v[c * per_step + i].T)
            for j in range(n_tile):
                k_s[j, 0:A_HALO, :] = k_s[j, A_CHUNK:, :]
            v_tail = [v_s[j, A_CHUNK:, :] for j in range(n_tile)]
            for u0 in range(0, A_CHUNK, A_UNIT):
                x = xa_v[pl.ds(r0 + u0, A_UNIT), :]
                k = _dot_nt(x, _unpack(wa_p[1]))
                for j in range(n_tile):
                    k_s[j, A_HALO + u0:A_HALO + u0 + A_UNIT, :] = k[:, j * LANES:(j + 1) * LANES]
                q_s[u0:u0 + A_UNIT, :] = _dot_nt(x, _unpack(wa_p[0])) * (a_scale * LOG2E)
                v = _dot_nt(x, _unpack(wa_p[2]))
                for j in range(n_tile):
                    vj = v[:, j * LANES:(j + 1) * LANES]
                    v_s[j, A_HALO + u0:A_HALO + u0 + A_UNIT, :] = vj
                    if u0 == 0:
                        first = jnp.broadcast_to(vj[0:1], (A_HALO, LANES))
                        v_s[j, 0:A_HALO, :] = jnp.where(c == 0, first, v_tail[j])
                for b0 in range(u0, u0 + A_UNIT, A_ROWS):
                    a_attend(b0, r0)
            for u0 in range(0, A_CHUNK, A_UNIT):
                y = _dot(oa_s[u0:u0 + A_UNIT, :], _unpack(wa_p[3]))
                outa_v[pl.ds(r0 + u0, A_UNIT), :] = y.astype(BF16)
            return carry

        with jax.named_scope('A'):
            lax.fori_loop(0, n_chunk, a_body, 0)

        outa_copy = pltpu.make_async_copy(outa_v, out_hbm.at[:, pl.ds(0, D)], sem_out.at[0])

        row = lax.broadcasted_iota(jnp.int32, (L, LANES), 0)
        lane = lax.broadcasted_iota(jnp.int32, (L, LANES), 1)
        key = jnp.where(lane < L, lane, lane - L)
        visible = (row < M) | (row >= key)
        in0 = lane < L
        in1 = (lane >= L) & (lane < 2 * L)
        fill0 = jnp.where(in0, NEG * LOG2E, -jnp.inf).astype(F32)
        fill1 = jnp.where(in1, NEG * LOG2E, -jnp.inf).astype(F32)
        split = Dh - LANES
        lo = lane < split

        def block_diag(t):
            z = jnp.zeros((L, LANES), F32)
            mid = t[:, LANES:2 * LANES]
            top = jnp.concatenate([t[:, :LANES], jnp.where(lo, mid, 0.0), z], axis=1)
            bot = jnp.concatenate([z, jnp.where(lo, 0.0, mid), t[:, 2 * LANES:]], axis=1)
            pad = jnp.zeros((LANES - 2 * L, PW), F32)
            return jnp.concatenate([top, bot, pad], axis=0).astype(BF16)

        def softmax2(s):
            s = s * (b_scale * LOG2E)
            s0 = jnp.where(visible & in0, s, fill0)
            s1 = jnp.where(visible & in1, s, fill1)
            m0 = jnp.max(s0, axis=1, keepdims=True)
            m1 = jnp.max(s1, axis=1, keepdims=True)
            e = jnp.exp2(jnp.where(in0, s0 - m0, s1 - m1))
            d0 = jnp.sum(jnp.where(in0, e, 0.0), axis=1, keepdims=True)
            d1 = jnp.sum(jnp.where(in0, 0.0, e), axis=1, keepdims=True)
            return e / jnp.where(in0, d0, d1)

        def outb_copy(r0):
            return pltpu.make_async_copy(
                outb_v.at[pl.ds(r0, seg)], out_hbm.at[pl.ds(r0, seg), pl.ds(D, D)], sem_out.at[1])

        def out_proj(p0, p1):
            w = _unpack(wo_p[p0:p1].reshape((p1 - p0) * PW // 2, D))
            return _dot(o_s[:, p0 * PW:p1 * PW], w)

        def attend(r0, with_head):
            h_s[M:, :] = xb_v[pl.ds(r0, seg), :].astype(F32)
            prob = vbd = acc = None
            for p in range(n_pair):
                h = h_s[...]
                if p == 0:
                    c0 = D - LANES
                    k = _dot(h[:, c0:], _unpack(w_p[n_spare + 3 * p + 0, c0 // 2:]))
                    q = _dot(h[:, c0:], _unpack(w_p[n_spare + 3 * p + 1, c0 // 2:]))
                    k = k + _dot(h[:, :c0], _unpack(w_p[n_spare + 3 * p + 0, :c0 // 2]))
                    q = q + _dot(h[:, :c0], _unpack(w_p[n_spare + 3 * p + 1, :c0 // 2]))
                else:
                    k = _dot(h, _unpack(w_p[n_spare + 3 * p + 0]))
                    q = _dot(h, _unpack(w_p[n_spare + 3 * p + 1]))
                v = _dot(h, _unpack(w_p[n_spare + 3 * p + 2]))
                if p > 0:
                    o_s[:, (p - 1) * PW:p * PW] = _dot(prob, vbd)
                if with_head and p == n_pair - 1:
                    acc = out_proj(0, 2)
                prob = softmax2(_dot_nt(q, block_diag(k)))
                vbd = block_diag(v)
            if with_head:
                acc = acc + out_proj(2, HEAD_PAIRS - 1)
            o_s[:, (n_pair - 1) * PW:] = _dot(prob, vbd)
            if with_head:
                acc_s[...] = acc + out_proj(HEAD_PAIRS - 1, HEAD_PAIRS)

        def finish(r0):
            acc = acc_s[...] + out_proj(HEAD_PAIRS, n_pair)
            h_s[0:M, :] = acc[0:M]
            outb_v[pl.ds(r0, seg), :] = acc[M:].astype(BF16)
            outb_copy(r0).start()

        with jax.named_scope('wait_xb'):
            mem_copy.wait()
            xb_head.wait()
        h_s[0:M, :] = mem0_v[...].astype(F32)
        attend(0, False)

        n_head = HEAD_PAIRS // pairs_per_wo
        with jax.named_scope('wo_wait'):
            for c in range(n_head):
                wo_copy(c).wait()
        w = wob_v[0:HEAD_PAIRS * PW, :]
        wo_p[0:HEAD_PAIRS] = _pack(w).reshape(HEAD_PAIRS, PW // 2, D)
        acc_s[...] = _dot(o_s[:, 0:HEAD_PAIRS * PW], w)

        def wo_tail(c, carry):
            wo_copy(c).wait()
            w = wob_v[pl.ds(pl.multiple_of(c * pairs_per_wo * PW, PW), pairs_per_wo * PW), :]
            wo_p[pl.ds(c * pairs_per_wo, pairs_per_wo)] = _pack(w).reshape(pairs_per_wo, PW // 2, D)
            return carry

        with jax.named_scope('wo'):
            lax.fori_loop(n_head, WO_CHUNKS, wo_tail, 0)
        outa_copy.start()

        def seg_body(i, carry):
            @pl.when(i == 1)
            def _():
                xb_rest.wait()

            for u in range(UNROLL):
                r0 = pl.multiple_of((i * UNROLL + u) * seg, seg)
                finish(r0)
                attend(pl.multiple_of(r0 + seg, seg), True)
            return carry

        with jax.named_scope('B'):
            lax.fori_loop(0, (n_seg - 1) // UNROLL, seg_body, 0)
        finish((n_seg - 1) * seg)

        outa_copy.wait()
        pltpu.make_async_copy(outb_v, outb_v, sem_out.at[1]).wait()

    scratch = [
        pltpu.VMEM((S, D), BF16),
        pltpu.VMEM((3, D, D), BF16),
        pltpu.VMEM((D, D), BF16),
        pltpu.VMEM((S, D), BF16),
        pltpu.VMEM((M, D), BF16),
        pltpu.VMEM((n_chunk * per_step, PW, D), BF16),
        pltpu.VMEM((H * Dh, D), BF16),
        pltpu.VMEM((n_tile, D // 2, LANES), jnp.int32),
        pltpu.VMEM((4, D // 2, D), jnp.int32),
        pltpu.VMEM((A_CHUNK, D), F32),
        pltpu.VMEM((n_tile, A_HALO + A_CHUNK, LANES), F32),
        pltpu.VMEM((n_tile, A_HALO + A_CHUNK, LANES), F32),
        pltpu.VMEM((A_CHUNK, D), F32),
        pltpu.VMEM((S, D), BF16),
        pltpu.VMEM((n_chunk * per_step, D // 2, PW), jnp.int32),
        pltpu.VMEM((n_pair, PW // 2, D), jnp.int32),
        pltpu.VMEM((L, D), F32),
        pltpu.VMEM((L, H * Dh), F32),
        pltpu.VMEM((L, D), F32),
        pltpu.VMEM((S, D), BF16),
        pltpu.SemaphoreType.DMA((7 + WO_CHUNKS + 2 * n_chunk,)),
        pltpu.SemaphoreType.DMA((2,)),
    ]
    return kernel, scratch


def pallas_concat_heads__sliding_local_dilated__memory_aug_recurrent_mem_tr__prompt_kernel(
    A_x, A_wqkv, A_wo, B_x, B_mem0, B_Wq, B_Wk, B_Wv, B_Wo, B_seg_len,
):
    _, S, D = A_x.shape
    _, H, Dh = B_Wq.shape
    M = B_mem0.shape[1]
    seg = int(B_seg_len)
    kernel, scratch = _make_kernel(S, D, H, Dh, M, seg)

    def rows_first(w):
        return jnp.transpose(w, (1, 2, 0)).reshape(H * Dh, D)

    out = pl.pallas_call(
        kernel,
        out_shape=jax.ShapeDtypeStruct((S, 2 * D), BF16),
        in_specs=[pl.BlockSpec(memory_space=pl.ANY)] * 9,
        out_specs=pl.BlockSpec(memory_space=pl.ANY),
        scratch_shapes=scratch,
        compiler_params=pltpu.CompilerParams(vmem_limit_bytes=110 * 2**20),
    )(
        A_x.reshape(S, D), A_wqkv, A_wo, B_x.reshape(S, D), B_mem0.reshape(M, D),
        rows_first(B_Wq), rows_first(B_Wk), rows_first(B_Wv), B_Wo.reshape(H * Dh, D),
    )
    return out.reshape(1, S, 2 * D)
```

```python
import jax
import jax.numpy as jnp
import numpy as np
from jax import lax
import jax.experimental.pallas as pl
import jax.experimental.pallas.tpu as pltpu

F32 = jnp.float32
BF16 = jnp.bfloat16
LANES = 128
NEG = -1000000000.0
LOG2E = float(np.log2(np.e))

A_HEADS = 32
A_WINDOW = 8
A_DILATION = 2
A_HALO = 16
A_CHUNK = 256
A_UNIT = 64
A_ROWS = 8
WO_CHUNKS = 2
UNROLL = 3
XB_HEAD = 32 * (UNROLL + 1)
HEAD_PAIRS = 4


def _dot(a, b):
    return lax.dot_general(a, b, (((1,), (0,)), ((), ())), preferred_element_type=F32)


def _dot_nt(a, b):
    return lax.dot_general(a, b, (((1,), (1,)), ((), ())), preferred_element_type=F32)


def _pack(w):
    return pltpu.bitcast(w, jnp.int32)


def _unpack(w):
    return pltpu.bitcast(w, BF16)


def _make_kernel(S, D, H, Dh, M, seg):
    n_seg = S // seg
    L = M + seg
    n_pair = H // 2
    PW = 2 * Dh
    n_tile = D // LANES
    n_chunk = S // A_CHUNK
    per_step = -(-3 * n_pair // (n_chunk - 1))
    n_spare = per_step * n_chunk - 3 * n_pair
    a_dh = D // A_HEADS
    a_scale = float(a_dh) ** -0.5
    b_scale = float(Dh) ** -0.5

    def kernel(xa_hbm, wqkv_hbm, woa_hbm, xb_hbm, mem0_hbm, wqt_hbm, wkt_hbm, wvt_hbm, wob_hbm,
               out_hbm,
               xa_v, wqkv_v, woa_v, xb_v, mem0_v, wt_v, wob_v,
               perm_s, wa_p, q_s, k_s, v_s, oa_s, outa_v,
               w_p, h_s, o_s, acc_s, outb_v,
               sem_in, sem_out):
        def wa_copy(t):
            if t == 3:
                return pltpu.make_async_copy(woa_hbm, woa_v, sem_in.at[3])
            return pltpu.make_async_copy(wqkv_hbm.at[:, pl.ds(t * D, D)], wqkv_v.at[t], sem_in.at[t])

        def xa_copy(c):
            rows = pl.ds(c * A_CHUNK, A_CHUNK)
            return pltpu.make_async_copy(xa_hbm.at[rows], xa_v.at[rows], sem_in.at[7 + WO_CHUNKS + c])

        def w_start(n):
            src = (wkt_hbm, wqt_hbm, wvt_hbm)[n % 3]
            pltpu.make_async_copy(src.at[pl.ds(n // 3 * PW, PW)], wt_v.at[n + n_spare],
                                  sem_in.at[7 + WO_CHUNKS + n_chunk + (n + n_spare) // per_step]).start()

        def w_wait(c, n):
            blocks = wt_v.at[pl.ds(0, n)]
            pltpu.make_async_copy(blocks, blocks, sem_in.at[7 + WO_CHUNKS + n_chunk + c]).wait()

        def wo_copy(p0, p1, slot):
            rows = pl.ds(p0 * PW, (p1 - p0) * PW)
            return pltpu.make_async_copy(wob_hbm.at[rows], wob_v.at[rows], sem_in.at[6 + slot])

        wo_head = wo_copy(0, HEAD_PAIRS, 0)
        wo_rest = wo_copy(HEAD_PAIRS, n_pair, 1)
        xb_head = pltpu.make_async_copy(xb_hbm.at[pl.ds(0, XB_HEAD)], xb_v.at[pl.ds(0, XB_HEAD)], sem_in.at[4])
        xb_rest = pltpu.make_async_copy(
            xb_hbm.at[pl.ds(XB_HEAD, S - XB_HEAD)], xb_v.at[pl.ds(XB_HEAD, S - XB_HEAD)], sem_in.at[6 + WO_CHUNKS])
        mem_copy = pltpu.make_async_copy(mem0_hbm, mem0_v, sem_in.at[5])

        for t in range(4):
            wa_copy(t).start()
        xa_copy(0).start()
        for c in range(1, n_chunk):
            xa_copy(c).start()
            for n in range(max(c * per_step - n_spare, 0), (c + 1) * per_step - n_spare):
                w_start(n)
        mem_copy.start()
        xb_head.start()
        wo_head.start()
        wo_rest.start()
        xb_rest.start()

        def store_reordered(t, w):
            w = _pack(w)
            for j in range(n_tile):
                perm_s[j] = w[:, j * LANES:(j + 1) * LANES]
            for dd in range(a_dh // 2):
                for j in range(n_tile):
                    u = perm_s[j, pl.ds(dd, A_HEADS, stride=a_dh // 2), :]
                    even = pltpu.bitcast(u << 16, F32)
                    odd = pltpu.bitcast(u & jnp.int32(-65536), F32)
                    both = jnp.concatenate([even, odd], axis=0).astype(BF16)
                    wa_p[t, dd * A_HEADS:(dd + 1) * A_HEADS, j * LANES:(j + 1) * LANES] = _pack(both)

        for t in range(3):
            wa_copy(t).wait()
            store_reordered(t, wqkv_v[t].T)
            wa_p[t] = _pack(_unpack(wa_p[t]).T)
        wa_copy(3).wait()
        store_reordered(3, woa_v[...])
        for j in range(n_tile):
            k_s[j, A_CHUNK:, :] = jnp.zeros((A_HALO, LANES), F32)
            v_s[j, A_CHUNK:, :] = jnp.zeros((A_HALO, LANES), F32)

        def a_attend(b0, r0):
            q = [q_s[b0:b0 + A_ROWS, j * LANES:(j + 1) * LANES] for j in range(n_tile)]
            logits = []
            for w in range(A_WINDOW):
                a0 = A_HALO + b0 - w * A_DILATION
                t = q[0] * k_s[0, a0:a0 + A_ROWS, :]
                for j in range(1, n_tile):
                    t = t + q[j] * k_s[j, a0:a0 + A_ROWS, :]
                t = t + pltpu.roll(t, 64, 1)
                t = t + pltpu.roll(t, 32, 1)
                if b0 < w * A_DILATION:
                    pos = r0 + b0 + lax.broadcasted_iota(jnp.int32, (A_ROWS, LANES), 0)
                    t = jnp.where(pos >= w * A_DILATION, t, NEG * LOG2E)
                logits.append(t)
            mx = logits[0]
            for t in logits[1:]:
                mx = jnp.maximum(mx, t)
            e = [jnp.exp2(t - mx) for t in logits]
            den = e[0]
            for t in e[1:]:
                den = den + t
            inv = 1.0 / den
            for j in range(n_tile):
                acc = e[0] * v_s[j, A_HALO + b0:A_HALO + b0 + A_ROWS, :]
                for w in range(1, A_WINDOW):
                    a0 = A_HALO + b0 - w * A_DILATION
                    acc = acc + e[w] * v_s[j, a0:a0 + A_ROWS, :]
                oa_s[b0:b0 + A_ROWS, j * LANES:(j + 1) * LANES] = acc * inv

        def a_body(c, carry):
            r0 = pl.multiple_of(c * A_CHUNK, A_CHUNK)
            xa_copy(c).wait()

            @pl.when(c == 1)
            def _():
                w_wait(c, 2 * per_step - n_spare)

            @pl.when(c > 1)
            def _():
                w_wait(c, per_step)

            for i in range(per_step):
                w_p[c * per_step + i] = _pack(wt_v[c * per_step + i].T)
            for j in range(n_tile):
                k_s[j, 0:A_HALO, :] = k_s[j, A_CHUNK:, :]
            v_tail = [v_s[j, A_CHUNK:, :] for j in range(n_tile)]
            for u0 in range(0, A_CHUNK, A_UNIT):
                x = xa_v[pl.ds(r0 + u0, A_UNIT), :]
                k = _dot(x, _unpack(wa_p[1]))
                for j in range(n_tile):
                    k_s[j, A_HALO + u0:A_HALO + u0 + A_UNIT, :] = k[:, j * LANES:(j + 1) * LANES]
                q_s[u0:u0 + A_UNIT, :] = _dot(x, _unpack(wa_p[0])) * (a_scale * LOG2E)
                v = _dot(x, _unpack(wa_p[2]))
                for j in range(n_tile):
                    vj = v[:, j * LANES:(j + 1) * LANES]
                    v_s[j, A_HALO + u0:A_HALO + u0 + A_UNIT, :] = vj
                    if u0 == 0:
                        first = jnp.broadcast_to(vj[0:1], (A_HALO, LANES))
                        v_s[j, 0:A_HALO, :] = jnp.where(c == 0, first, v_tail[j])
                for b0 in range(u0, u0 + A_UNIT, A_ROWS):
                    a_attend(b0, r0)
            for u0 in range(0, A_CHUNK, A_UNIT):
                y = _dot(oa_s[u0:u0 + A_UNIT, :], _unpack(wa_p[3]))
                outa_v[pl.ds(r0 + u0, A_UNIT), :] = y.astype(BF16)
            return carry

        with jax.named_scope('A'):
            lax.fori_loop(0, n_chunk, a_body, 0)

        outa_copy = pltpu.make_async_copy(outa_v, out_hbm.at[:, pl.ds(0, D)], sem_out.at[0])

        row = lax.broadcasted_iota(jnp.int32, (L, LANES), 0)
        lane = lax.broadcasted_iota(jnp.int32, (L, LANES), 1)
        key = jnp.where(lane < L, lane, lane - L)
        visible = (row < M) | (row >= key)
        in0 = lane < L
        in1 = (lane >= L) & (lane < 2 * L)
        fill0 = jnp.where(in0, NEG * LOG2E, -jnp.inf).astype(F32)
        fill1 = jnp.where(in1, NEG * LOG2E, -jnp.inf).astype(F32)
        split = Dh - LANES
        lo = lane < split

        def block_diag(t):
            z = jnp.zeros((L, LANES), F32)
            mid = t[:, LANES:2 * LANES]
            top = jnp.concatenate([t[:, :LANES], jnp.where(lo, mid, 0.0), z], axis=1)
            bot = jnp.concatenate([z, jnp.where(lo, 0.0, mid), t[:, 2 * LANES:]], axis=1)
            pad = jnp.zeros((LANES - 2 * L, PW), F32)
            return jnp.concatenate([top, bot, pad], axis=0).astype(BF16)

        def softmax2(s):
            s = s * (b_scale * LOG2E)
            s0 = jnp.where(visible & in0, s, fill0)
            s1 = jnp.where(visible & in1, s, fill1)
            m0 = jnp.max(s0, axis=1, keepdims=True)
            m1 = jnp.max(s1, axis=1, keepdims=True)
            e = jnp.exp2(jnp.where(in0, s0 - m0, s1 - m1))
            d0 = jnp.sum(jnp.where(in0, e, 0.0), axis=1, keepdims=True)
            d1 = jnp.sum(jnp.where(in0, 0.0, e), axis=1, keepdims=True)
            return e / jnp.where(in0, d0, d1)

        def outb_copy(r0):
            return pltpu.make_async_copy(
                outb_v.at[pl.ds(r0, seg)], out_hbm.at[pl.ds(r0, seg), pl.ds(D, D)], sem_out.at[1])

        def out_proj(p0, p1):
            w = wob_v[p0 * PW:p1 * PW, :]
            return _dot(o_s[:, p0 * PW:p1 * PW], w)

        def attend(r0):
            h_s[M:, :] = xb_v[pl.ds(r0, seg), :].astype(F32)
            prob = vbd = acc = None
            for p in range(n_pair):
                h = h_s[...]
                if p == 0:
                    c0 = D - LANES
                    k = _dot(h[:, c0:], _unpack(w_p[n_spare + 3 * p + 0, c0 // 2:]))
                    q = _dot(h[:, c0:], _unpack(w_p[n_spare + 3 * p + 1, c0 // 2:]))
                    k = k + _dot(h[:, :c0], _unpack(w_p[n_spare + 3 * p + 0, :c0 // 2]))
                    q = q + _dot(h[:, :c0], _unpack(w_p[n_spare + 3 * p + 1, :c0 // 2]))
                else:
                    k = _dot(h, _unpack(w_p[n_spare + 3 * p + 0]))
                    q = _dot(h, _unpack(w_p[n_spare + 3 * p + 1]))
                v = _dot(h, _unpack(w_p[n_spare + 3 * p + 2]))
                if p > 0:
                    o_s[:, (p - 1) * PW:p * PW] = _dot(prob, vbd)
                if p == n_pair - 1:
                    acc = out_proj(0, 1)
                prob = softmax2(_dot_nt(q, block_diag(k)))
                vbd = block_diag(v)
            acc_s[...] = acc + out_proj(1, HEAD_PAIRS)
            o_s[:, (n_pair - 1) * PW:] = _dot(prob, vbd)

        def finish(r0):
            acc = acc_s[...] + out_proj(HEAD_PAIRS, n_pair)
            h_s[0:M, :] = acc[0:M]
            outb_v[pl.ds(r0, seg), :] = acc[M:].astype(BF16)
            outb_copy(r0).start()

        with jax.named_scope('wait_xb'):
            mem_copy.wait()
            xb_head.wait()
            wo_head.wait()
        h_s[0:M, :] = mem0_v[...].astype(F32)
        attend(0)

        with jax.named_scope('wo_wait'):
            wo_rest.wait()
        outa_copy.start()

        def seg_body(i, carry):
            @pl.when(i == 1)
            def _():
                xb_rest.wait()

            for u in range(UNROLL):
                r0 = pl.multiple_of((i * UNROLL + u) * seg, seg)
                finish(r0)
                attend(pl.multiple_of(r0 + seg, seg))
            return carry

        with jax.named_scope('B'):
            lax.fori_loop(0, (n_seg - 1) // UNROLL, seg_body, 0)
        finish((n_seg - 1) * seg)

        outa_copy.wait()
        pltpu.make_async_copy(outb_v, outb_v, sem_out.at[1]).wait()

    scratch = [
        pltpu.VMEM((S, D), BF16),
        pltpu.VMEM((3, D, D), BF16),
        pltpu.VMEM((D, D), BF16),
        pltpu.VMEM((S, D), BF16),
        pltpu.VMEM((M, D), BF16),
        pltpu.VMEM((n_chunk * per_step, PW, D), BF16),
        pltpu.VMEM((H * Dh, D), BF16),
        pltpu.VMEM((n_tile, D // 2, LANES), jnp.int32),
        pltpu.VMEM((4, D // 2, D), jnp.int32),
        pltpu.VMEM((A_CHUNK, D), F32),
        pltpu.VMEM((n_tile, A_HALO + A_CHUNK, LANES), F32),
        pltpu.VMEM((n_tile, A_HALO + A_CHUNK, LANES), F32),
        pltpu.VMEM((A_CHUNK, D), F32),
        pltpu.VMEM((S, D), BF16),
        pltpu.VMEM((n_chunk * per_step, D // 2, PW), jnp.int32),
        pltpu.VMEM((L, D), F32),
        pltpu.VMEM((L, H * Dh), F32),
        pltpu.VMEM((L, D), F32),
        pltpu.VMEM((S, D), BF16),
        pltpu.SemaphoreType.DMA((7 + WO_CHUNKS + 2 * n_chunk,)),
        pltpu.SemaphoreType.DMA((2,)),
    ]
    return kernel, scratch


def pallas_concat_heads__sliding_local_dilated__memory_aug_recurrent_mem_tr__prompt_kernel(
    A_x, A_wqkv, A_wo, B_x, B_mem0, B_Wq, B_Wk, B_Wv, B_Wo, B_seg_len,
):
    _, S, D = A_x.shape
    _, H, Dh = B_Wq.shape
    M = B_mem0.shape[1]
    seg = int(B_seg_len)
    kernel, scratch = _make_kernel(S, D, H, Dh, M, seg)

    def rows_first(w):
        return jnp.transpose(w, (1, 2, 0)).reshape(H * Dh, D)

    out = pl.pallas_call(
        kernel,
        out_shape=jax.ShapeDtypeStruct((S, 2 * D), BF16),
        in_specs=[pl.BlockSpec(memory_space=pl.ANY)] * 9,
        out_specs=pl.BlockSpec(memory_space=pl.ANY),
        scratch_shapes=scratch,
        compiler_params=pltpu.CompilerParams(vmem_limit_bytes=110 * 2**20),
    )(
        A_x.reshape(S, D), A_wqkv, A_wo, B_x.reshape(S, D), B_mem0.reshape(M, D),
        rows_first(B_Wq), rows_first(B_Wk), rows_first(B_Wv), B_Wo.reshape(H * Dh, D),
    )
    return out.reshape(1, S, 2 * D)
```

```python
import functools

import jax
import jax.numpy as jnp
import numpy as np
from jax import lax
import jax.experimental.pallas as pl
import jax.experimental.pallas.tpu as pltpu

F32 = jnp.float32
BF16 = jnp.bfloat16
LANES = 128
LOG2E = float(np.log2(np.e))
MASKED = -1000000000.0 * LOG2E

A_HEADS = 32
A_WINDOW = 8
A_DILATION = 2
A_HALO = 16
A_CHUNK = 256
A_UNIT = 64
A_ROWS = 8

B_UNROLL = 3
B_HEAD_PAIRS = 4


def _dot(a, b):
    return lax.dot_general(a, b, (((1,), (0,)), ((), ())), preferred_element_type=F32)


def _dot_nt(a, b):
    return lax.dot_general(a, b, (((1,), (1,)), ((), ())), preferred_element_type=F32)


def _pack(w):
    return pltpu.bitcast(w, jnp.int32)


def _unpack(w):
    return pltpu.bitcast(w, BF16)


def _block(i, size):
    start = i * size
    return pl.ds(start if isinstance(start, int) else pl.multiple_of(start, size), size)


def _make_kernel(S, D, H, Dh, M, seg):
    n_seg = S // seg
    L = M + seg
    n_pair = H // 2
    PW = 2 * Dh
    n_tile = D // LANES
    n_chunk = S // A_CHUNK
    a_dh = D // A_HEADS
    a_scale = float(a_dh) ** -0.5
    b_scale = float(Dh) ** -0.5
    assert D % LANES == 0 and a_dh % 2 == 0 and 4 * A_HEADS == LANES and S % A_CHUNK == 0
    assert PW == 3 * LANES and H % 2 == 0 and M % 8 == 0 and seg % 16 == 0 and 2 * L < LANES
    assert S % seg == 0 and (n_seg - 1) % B_UNROLL == 0 and n_seg - 1 > B_UNROLL

    per_step = pl.cdiv(3 * n_pair, n_chunk - 1)
    n_spare = per_step * n_chunk - 3 * n_pair
    xb_head_rows = seg * (B_UNROLL + 1)

    SEM_MEM, SEM_XB, SEM_WO, SEM_XA = 4, 5, 7, 9
    SEM_W = SEM_XA + n_chunk

    def kernel(xa_hbm, wqkv_hbm, woa_hbm, xb_hbm, mem0_hbm, wqt_hbm, wkt_hbm, wvt_hbm, wob_hbm,
               out_hbm,
               xa_v, wqkv_v, woa_v, xb_v, mem0_v, wt_v, wob_v,
               perm_s, wa_p, q_s, k_s, v_s, oa_s, outa_v,
               w_p, h_s, o_s, acc_s, outb_v,
               sem_in, sem_out):
        def wa_copy(t):
            if t == 3:
                return pltpu.make_async_copy(woa_hbm, woa_v, sem_in.at[t])
            return pltpu.make_async_copy(wqkv_hbm.at[:, pl.ds(t * D, D)], wqkv_v.at[t], sem_in.at[t])

        def rows_copy(src, dst, rows, slot):
            return pltpu.make_async_copy(src.at[rows], dst.at[rows], sem_in.at[slot])

        def xa_copy(c):
            return rows_copy(xa_hbm, xa_v, _block(c, A_CHUNK), SEM_XA + c)

        def w_start(c):
            for t, src in enumerate((wkt_hbm, wqt_hbm, wvt_hbm)):
                first = n_spare + t * n_pair
                lo, hi = max(c * per_step, first), min((c + 1) * per_step, first + n_pair)
                if lo < hi:
                    pltpu.make_async_copy(
                        src.at[pl.ds((lo - first) * PW, (hi - lo) * PW)],
                        wt_v.at[pl.ds(lo * PW, (hi - lo) * PW)], sem_in.at[SEM_W + c]).start()

        def w_wait(c, rows):
            pltpu.make_async_copy(wt_v.at[rows], wt_v.at[rows], sem_in.at[SEM_W + c]).wait()

        mem_copy = pltpu.make_async_copy(mem0_hbm, mem0_v, sem_in.at[SEM_MEM])
        xb_head = rows_copy(xb_hbm, xb_v, pl.ds(0, xb_head_rows), SEM_XB)
        xb_rest = rows_copy(xb_hbm, xb_v, pl.ds(xb_head_rows, S - xb_head_rows), SEM_XB + 1)
        wo_head = rows_copy(wob_hbm, wob_v, pl.ds(0, B_HEAD_PAIRS * PW), SEM_WO)
        wo_rest = rows_copy(
            wob_hbm, wob_v, pl.ds(B_HEAD_PAIRS * PW, (n_pair - B_HEAD_PAIRS) * PW), SEM_WO + 1)
        outa_copy = pltpu.make_async_copy(outa_v, out_hbm.at[:, pl.ds(0, D)], sem_out.at[0])

        def outb_copy(rows):
            return pltpu.make_async_copy(outb_v.at[rows], out_hbm.at[rows, pl.ds(D, D)], sem_out.at[1])

        for t in range(4):
            wa_copy(t).start()
        for c in range(n_chunk):
            xa_copy(c).start()
            w_start(c)
        for cp in (mem_copy, xb_head, wo_head, wo_rest, xb_rest):
            cp.start()

        def reorder_features(t, w):
            w = _pack(w)
            for j in range(n_tile):
                perm_s[j] = w[:, j * LANES:(j + 1) * LANES]
            for dd in range(a_dh // 2):
                for j in range(n_tile):
                    u = perm_s[j, pl.ds(dd, A_HEADS, stride=a_dh // 2), :]
                    even = pltpu.bitcast(u << 16, F32)
                    odd = pltpu.bitcast(u & jnp.int32(-65536), F32)
                    both = jnp.concatenate([even, odd], axis=0).astype(BF16)
                    wa_p[t, dd * A_HEADS:(dd + 1) * A_HEADS, j * LANES:(j + 1) * LANES] = _pack(both)

        for t in range(3):
            wa_copy(t).wait()
            reorder_features(t, wqkv_v[t].T)
            wa_p[t] = _pack(_unpack(wa_p[t]).T)
        wa_copy(3).wait()
        reorder_features(3, woa_v[...])
        for j in range(n_tile):
            k_s[j, A_CHUNK:, :] = jnp.zeros((A_HALO, LANES), F32)
            v_s[j, A_CHUNK:, :] = jnp.zeros((A_HALO, LANES), F32)

        def a_attend(c, b0):
            def shifted(ref, j, w):
                start = A_HALO + b0 - w * A_DILATION
                return ref[j, start:start + A_ROWS, :]

            q = [q_s[b0:b0 + A_ROWS, j * LANES:(j + 1) * LANES] for j in range(n_tile)]
            logits = []
            for w in range(A_WINDOW):
                t = q[0] * shifted(k_s, 0, w)
                for j in range(1, n_tile):
                    t = t + q[j] * shifted(k_s, j, w)
                t = t + pltpu.roll(t, 2 * A_HEADS, 1)
                t = t + pltpu.roll(t, A_HEADS, 1)
                if b0 < w * A_DILATION:
                    pos = c * A_CHUNK + b0 + lax.broadcasted_iota(jnp.int32, (A_ROWS, LANES), 0)
                    t = jnp.where(pos >= w * A_DILATION, t, MASKED)
                logits.append(t)
            top = functools.reduce(jnp.maximum, logits)
            e = [jnp.exp2(t - top) for t in logits]
            inv = 1.0 / functools.reduce(jnp.add, e)
            for j in range(n_tile):
                acc = e[0] * shifted(v_s, j, 0)
                for w in range(1, A_WINDOW):
                    acc = acc + e[w] * shifted(v_s, j, w)
                oa_s[b0:b0 + A_ROWS, j * LANES:(j + 1) * LANES] = acc * inv

        def a_step(c, carry):
            xa_copy(c).wait()
            c_first, skip = divmod(n_spare, per_step)

            @pl.when(c == c_first)
            def _():
                w_wait(c_first, pl.ds(n_spare * PW, (per_step - skip) * PW))

            @pl.when(c > c_first)
            def _():
                w_wait(c, _block(c, per_step * PW))

            for i in range(per_step):
                slot = c * per_step + i
                w_p[slot] = _pack(wt_v[_block(slot, PW), :].T)

            for j in range(n_tile):
                k_s[j, 0:A_HALO, :] = k_s[j, A_CHUNK:, :]
            v_tail = [v_s[j, A_CHUNK:, :] for j in range(n_tile)]
            units = A_CHUNK // A_UNIT
            for u in range(units):
                u0 = u * A_UNIT
                x = xa_v[_block(c * units + u, A_UNIT), :]
                k = _dot(x, _unpack(wa_p[1]))
                for j in range(n_tile):
                    k_s[j, A_HALO + u0:A_HALO + u0 + A_UNIT, :] = k[:, j * LANES:(j + 1) * LANES]
                q_s[u0:u0 + A_UNIT, :] = _dot(x, _unpack(wa_p[0])) * (a_scale * LOG2E)
                v = _dot(x, _unpack(wa_p[2]))
                for j in range(n_tile):
                    vj = v[:, j * LANES:(j + 1) * LANES]
                    v_s[j, A_HALO + u0:A_HALO + u0 + A_UNIT, :] = vj
                    if u == 0:
                        row0 = jnp.broadcast_to(vj[0:1], (A_HALO, LANES))
                        v_s[j, 0:A_HALO, :] = jnp.where(c == 0, row0, v_tail[j])
                for b0 in range(u0, u0 + A_UNIT, A_ROWS):
                    a_attend(c, b0)
            for u in range(units):
                y = _dot(oa_s[u * A_UNIT:(u + 1) * A_UNIT, :], _unpack(wa_p[3]))
                outa_v[_block(c * units + u, A_UNIT), :] = y.astype(BF16)
            return carry

        lax.fori_loop(0, n_chunk, a_step, 0)

        row = lax.broadcasted_iota(jnp.int32, (L, LANES), 0)
        lane = lax.broadcasted_iota(jnp.int32, (L, LANES), 1)
        visible = (row < M) | (row >= jnp.where(lane < L, lane, lane - L))
        in0 = lane < L
        in1 = (lane >= L) & (lane < 2 * L)
        fill0 = jnp.where(in0, MASKED, -jnp.inf).astype(F32)
        fill1 = jnp.where(in1, MASKED, -jnp.inf).astype(F32)
        first_head = lane < Dh - LANES

        def block_diag(t):
            z = jnp.zeros((L, LANES), F32)
            mid = t[:, LANES:2 * LANES]
            top = jnp.concatenate([t[:, :LANES], jnp.where(first_head, mid, 0.0), z], axis=1)
            bot = jnp.concatenate([z, jnp.where(first_head, 0.0, mid), t[:, 2 * LANES:]], axis=1)
            pad = jnp.zeros((LANES - 2 * L, PW), F32)
            return jnp.concatenate([top, bot, pad], axis=0).astype(BF16)

        def pair_softmax(s):
            s = s * (b_scale * LOG2E)
            s0 = jnp.where(visible & in0, s, fill0)
            s1 = jnp.where(visible & in1, s, fill1)
            m0 = jnp.max(s0, axis=1, keepdims=True)
            m1 = jnp.max(s1, axis=1, keepdims=True)
            e = jnp.exp2(jnp.where(in0, s0 - m0, s1 - m1))
            d0 = jnp.sum(jnp.where(in0, e, 0.0), axis=1, keepdims=True)
            d1 = jnp.sum(jnp.where(in0, 0.0, e), axis=1, keepdims=True)
            return e / jnp.where(in0, d0, d1)

        def weight(t, p, k0=0, k1=D):
            return _unpack(w_p[n_spare + t * n_pair + p, k0 // 2:k1 // 2])

        def out_proj(p0, p1, r0=0):
            return _dot(o_s[r0:, p0 * PW:p1 * PW], wob_v[p0 * PW:p1 * PW, :])

        def attend(s):
            h_s[M:, :] = xb_v[_block(s, seg), :].astype(F32)
            prob = vbd = acc = None
            for p in range(n_pair):
                h = h_s[...]
                if p == 0:
                    c0 = D - LANES
                    k = _dot(h[:, c0:], weight(0, p, c0))
                    q = _dot(h[:, c0:], weight(1, p, c0))
                    k = k + _dot(h[:, :c0], weight(0, p, 0, c0))
                    q = q + _dot(h[:, :c0], weight(1, p, 0, c0))
                else:
                    k = _dot(h, weight(0, p))
                    q = _dot(h, weight(1, p))
                v = _dot(h, weight(2, p))
                if p > 0:
                    o_s[:, (p - 1) * PW:p * PW] = _dot(prob, vbd)
                if p == n_pair - 1:
                    acc = out_proj(0, 1)
                prob = pair_softmax(_dot_nt(q, block_diag(k)))
                vbd = block_diag(v)
            acc_s[...] = acc + out_proj(1, B_HEAD_PAIRS)
            o_s[:, (n_pair - 1) * PW:] = _dot(prob, vbd)

        def finish(s, last=False):
            if last:
                y = acc_s[M:, :] + out_proj(B_HEAD_PAIRS, n_pair, M)
            else:
                acc = acc_s[...] + out_proj(B_HEAD_PAIRS, n_pair)
                h_s[0:M, :] = acc[0:M]
                y = acc[M:]
            outb_v[_block(s, seg), :] = y.astype(BF16)
            outb_copy(_block(s, seg)).start()

        for cp in (mem_copy, xb_head, wo_head):
            cp.wait()
        h_s[0:M, :] = mem0_v[...].astype(F32)
        attend(0)
        wo_rest.wait()
        outa_copy.start()

        def b_step(i, carry):
            @pl.when(i == 1)
            def _():
                xb_rest.wait()

            for u in range(B_UNROLL):
                finish(i * B_UNROLL + u)
                attend(i * B_UNROLL + u + 1)
            return carry

        lax.fori_loop(0, (n_seg - 1) // B_UNROLL, b_step, 0)
        finish(n_seg - 1, last=True)

        outa_copy.wait()
        outb_copy(pl.ds(0, S)).wait()

    n_slot = per_step * n_chunk
    scratch = [
        pltpu.VMEM((S, D), BF16),
        pltpu.VMEM((3, D, D), BF16),
        pltpu.VMEM((D, D), BF16),
        pltpu.VMEM((S, D), BF16),
        pltpu.VMEM((M, D), BF16),
        pltpu.VMEM((n_slot * PW, D), BF16),
        pltpu.VMEM((H * Dh, D), BF16),
        pltpu.VMEM((n_tile, D // 2, LANES), jnp.int32),
        pltpu.VMEM((4, D // 2, D), jnp.int32),
        pltpu.VMEM((A_CHUNK, D), F32),
        pltpu.VMEM((n_tile, A_HALO + A_CHUNK, LANES), F32),
        pltpu.VMEM((n_tile, A_HALO + A_CHUNK, LANES), F32),
        pltpu.VMEM((A_CHUNK, D), F32),
        pltpu.VMEM((S, D), BF16),
        pltpu.VMEM((n_slot, D // 2, PW), jnp.int32),
        pltpu.VMEM((L, D), F32),
        pltpu.VMEM((L, H * Dh), F32),
        pltpu.VMEM((L, D), F32),
        pltpu.VMEM((S, D), BF16),
        pltpu.SemaphoreType.DMA((SEM_W + n_chunk,)),
        pltpu.SemaphoreType.DMA((2,)),
    ]
    return kernel, scratch


@functools.partial(jax.jit, static_argnames=("B_seg_len",))
def pallas_concat_heads__sliding_local_dilated__memory_aug_recurrent_mem_tr__prompt_kernel(
    A_x, A_wqkv, A_wo, B_x, B_mem0, B_Wq, B_Wk, B_Wv, B_Wo, B_seg_len,
):
    _, S, D = A_x.shape
    _, H, Dh = B_Wq.shape
    M = B_mem0.shape[1]
    kernel, scratch = _make_kernel(S, D, H, Dh, M, B_seg_len)

    def features_first(w):
        return jnp.transpose(w, (1, 2, 0)).reshape(H * Dh, D)

    out = pl.pallas_call(
        kernel,
        out_shape=jax.ShapeDtypeStruct((S, 2 * D), BF16),
        in_specs=[pl.BlockSpec(memory_space=pl.ANY)] * 9,
        out_specs=pl.BlockSpec(memory_space=pl.ANY),
        scratch_shapes=scratch,
        compiler_params=pltpu.CompilerParams(vmem_limit_bytes=100 * 2**20),
    )(
        A_x.reshape(S, D), A_wqkv, A_wo, B_x.reshape(S, D), B_mem0.reshape(M, D),
        features_first(B_Wq), features_first(B_Wk), features_first(B_Wv), B_Wo.reshape(H * Dh, D),
    )
    return out.reshape(1, S, 2 * D)
```

```python
import functools

import jax
import jax.numpy as jnp
import numpy as np
from jax import lax
import jax.experimental.pallas as pl
import jax.experimental.pallas.tpu as pltpu

F32 = jnp.float32
BF16 = jnp.bfloat16
LANES = 128
LOG2E = float(np.log2(np.e))
MASKED = -1000000000.0 * LOG2E

A_HEADS = 32
A_WINDOW = 8
A_DILATION = 2
A_HALO = 16
A_CHUNK = 256
A_UNIT = 64
A_ROWS = 8

B_UNROLL = 3
B_HEAD_PAIRS = 4


def _dot(a, b):
    return lax.dot_general(a, b, (((1,), (0,)), ((), ())), preferred_element_type=F32)


def _dot_nt(a, b):
    return lax.dot_general(a, b, (((1,), (1,)), ((), ())), preferred_element_type=F32)


def _pack(w):
    return pltpu.bitcast(w, jnp.int32)


def _unpack(w):
    return pltpu.bitcast(w, BF16)


def _block(i, size):
    start = i * size
    return pl.ds(start if isinstance(start, int) else pl.multiple_of(start, size), size)


def _make_kernel(S, D, H, Dh, M, seg):
    n_seg = S // seg
    L = M + seg
    n_pair = H // 2
    PW = 2 * Dh
    n_tile = D // LANES
    n_chunk = S // A_CHUNK
    a_dh = D // A_HEADS
    a_scale = float(a_dh) ** -0.5
    b_scale = float(Dh) ** -0.5
    assert D % LANES == 0 and a_dh % 2 == 0 and 4 * A_HEADS == LANES and S % A_CHUNK == 0
    assert PW == 3 * LANES and H % 2 == 0 and M % 8 == 0 and seg % 16 == 0 and 2 * L < LANES
    assert S % seg == 0 and (n_seg - 1) % B_UNROLL == 0 and n_seg - 1 > B_UNROLL

    per_step = pl.cdiv(3 * n_pair, n_chunk - 1)
    n_idle = per_step * n_chunk - 3 * n_pair
    xb_head_rows = seg * (B_UNROLL + 1)

    SEM_MEM, SEM_XB, SEM_WO, SEM_XA = 4, 5, 7, 9
    SEM_W = SEM_XA + n_chunk

    def kernel(xa_hbm, wqkv_hbm, woa_hbm, xb_hbm, mem0_hbm, wqt_hbm, wkt_hbm, wvt_hbm, wob_hbm,
               out_hbm,
               xa_v, wqkv_v, woa_v, xb_v, mem0_v, wt_v, wob_v,
               perm_s, wa_p, q_s, k_s, v_s, oa_s, outa_v,
               w_p, h_s, o_s, acc_s, outb_v,
               sem_in, sem_out):
        def wa_copy(t):
            if t == 3:
                return pltpu.make_async_copy(woa_hbm, woa_v, sem_in.at[t])
            return pltpu.make_async_copy(wqkv_hbm.at[:, pl.ds(t * D, D)], wqkv_v.at[t], sem_in.at[t])

        def rows_copy(src, dst, rows, slot):
            return pltpu.make_async_copy(src.at[rows], dst.at[rows], sem_in.at[slot])

        def xa_copy(c):
            return rows_copy(xa_hbm, xa_v, _block(c, A_CHUNK), SEM_XA + c)

        def w_start(c):
            for t, src in enumerate((wkt_hbm, wqt_hbm, wvt_hbm)):
                lo = max(c * per_step - n_idle, t * n_pair)
                hi = min((c + 1) * per_step - n_idle, (t + 1) * n_pair)
                if lo < hi:
                    pltpu.make_async_copy(
                        src.at[pl.ds((lo - t * n_pair) * PW, (hi - lo) * PW)],
                        wt_v.at[pl.ds((1 + lo) * PW, (hi - lo) * PW)], sem_in.at[SEM_W + c]).start()

        def w_wait(c, lo, n):
            rows = pl.ds((1 + lo) * PW, n * PW)
            pltpu.make_async_copy(wt_v.at[rows], wt_v.at[rows], sem_in.at[SEM_W + c]).wait()

        mem_copy = pltpu.make_async_copy(mem0_hbm, mem0_v, sem_in.at[SEM_MEM])
        xb_head = rows_copy(xb_hbm, xb_v, pl.ds(0, xb_head_rows), SEM_XB)
        xb_rest = rows_copy(xb_hbm, xb_v, pl.ds(xb_head_rows, S - xb_head_rows), SEM_XB + 1)
        wo_head = rows_copy(wob_hbm, wob_v, pl.ds(0, B_HEAD_PAIRS * PW), SEM_WO)
        wo_rest = rows_copy(
            wob_hbm, wob_v, pl.ds(B_HEAD_PAIRS * PW, (n_pair - B_HEAD_PAIRS) * PW), SEM_WO + 1)
        outa_copy = pltpu.make_async_copy(outa_v, out_hbm.at[:, pl.ds(0, D)], sem_out.at[0])

        def outb_copy(rows):
            return pltpu.make_async_copy(outb_v.at[rows], out_hbm.at[rows, pl.ds(D, D)], sem_out.at[1])

        for t in range(4):
            wa_copy(t).start()
        for c in range(n_chunk):
            xa_copy(c).start()
            w_start(c)
        for cp in (mem_copy, xb_head, wo_head, wo_rest, xb_rest):
            cp.start()
        wt_v[0:PW, :] = jnp.zeros((PW, D), BF16)

        def reorder_features(t, w):
            w = _pack(w)
            for j in range(n_tile):
                perm_s[j] = w[:, j * LANES:(j + 1) * LANES]
            for dd in range(a_dh // 2):
                for j in range(n_tile):
                    u = perm_s[j, pl.ds(dd, A_HEADS, stride=a_dh // 2), :]
                    even = pltpu.bitcast(u << 16, F32)
                    odd = pltpu.bitcast(u & jnp.int32(-65536), F32)
                    both = jnp.concatenate([even, odd], axis=0).astype(BF16)
                    wa_p[t, dd * A_HEADS:(dd + 1) * A_HEADS, j * LANES:(j + 1) * LANES] = _pack(both)

        for t in range(3):
            wa_copy(t).wait()
            reorder_features(t, wqkv_v[t].T)
            wa_p[t] = _pack(_unpack(wa_p[t]).T)
        wa_copy(3).wait()
        reorder_features(3, woa_v[...])
        for j in range(n_tile):
            k_s[j, A_CHUNK:, :] = jnp.zeros((A_HALO, LANES), F32)
            v_s[j, A_CHUNK:, :] = jnp.zeros((A_HALO, LANES), F32)

        def a_attend(c, b0):
            def shifted(ref, j, w):
                start = A_HALO + b0 - w * A_DILATION
                return ref[j, start:start + A_ROWS, :]

            q = [q_s[b0:b0 + A_ROWS, j * LANES:(j + 1) * LANES] for j in range(n_tile)]
            logits = []
            for w in range(A_WINDOW):
                t = q[0] * shifted(k_s, 0, w)
                for j in range(1, n_tile):
                    t = t + q[j] * shifted(k_s, j, w)
                t = t + pltpu.roll(t, 2 * A_HEADS, 1)
                t = t + pltpu.roll(t, A_HEADS, 1)
                if b0 < w * A_DILATION:
                    pos = c * A_CHUNK + b0 + lax.broadcasted_iota(jnp.int32, (A_ROWS, LANES), 0)
                    t = jnp.where(pos >= w * A_DILATION, t, MASKED)
                logits.append(t)
            top = functools.reduce(jnp.maximum, logits)
            e = [jnp.exp2(t - top) for t in logits]
            inv = 1.0 / functools.reduce(jnp.add, e)
            for j in range(n_tile):
                acc = e[0] * shifted(v_s, j, 0)
                for w in range(1, A_WINDOW):
                    acc = acc + e[w] * shifted(v_s, j, w)
                oa_s[b0:b0 + A_ROWS, j * LANES:(j + 1) * LANES] = acc * inv

        def a_step(c, carry):
            xa_copy(c).wait()
            c_first, skip = divmod(n_idle, per_step)

            @pl.when(c == c_first)
            def _():
                w_wait(c_first, 0, per_step - skip)

            @pl.when(c > c_first)
            def _():
                w_wait(c, c * per_step - n_idle, per_step)

            for i in range(per_step):
                slot = jnp.maximum(1 + c * per_step + i - n_idle, 0)
                w_p[slot] = _pack(wt_v[_block(slot, PW), :].T)

            for j in range(n_tile):
                k_s[j, 0:A_HALO, :] = k_s[j, A_CHUNK:, :]
            v_tail = [v_s[j, A_CHUNK:, :] for j in range(n_tile)]
            units = A_CHUNK // A_UNIT
            for u in range(units):
                u0 = u * A_UNIT
                x = xa_v[_block(c * units + u, A_UNIT), :]
                k = _dot(x, _unpack(wa_p[1]))
                for j in range(n_tile):
                    k_s[j, A_HALO + u0:A_HALO + u0 + A_UNIT, :] = k[:, j * LANES:(j + 1) * LANES]
                q_s[u0:u0 + A_UNIT, :] = _dot(x, _unpack(wa_p[0])) * (a_scale * LOG2E)
                v = _dot(x, _unpack(wa_p[2]))
                for j in range(n_tile):
                    vj = v[:, j * LANES:(j + 1) * LANES]
                    v_s[j, A_HALO + u0:A_HALO + u0 + A_UNIT, :] = vj
                    if u == 0:
                        row0 = jnp.broadcast_to(vj[0:1], (A_HALO, LANES))
                        v_s[j, 0:A_HALO, :] = jnp.where(c == 0, row0, v_tail[j])
                for b0 in range(u0, u0 + A_UNIT, A_ROWS):
                    a_attend(c, b0)
            for u in range(units):
                y = _dot(oa_s[u * A_UNIT:(u + 1) * A_UNIT, :], _unpack(wa_p[3]))
                outa_v[_block(c * units + u, A_UNIT), :] = y.astype(BF16)
            return carry

        lax.fori_loop(0, n_chunk, a_step, 0)

        row = lax.broadcasted_iota(jnp.int32, (L, LANES), 0)
        lane = lax.broadcasted_iota(jnp.int32, (L, LANES), 1)
        visible = (row < M) | (row >= jnp.where(lane < L, lane, lane - L))
        in0 = lane < L
        in1 = (lane >= L) & (lane < 2 * L)
        fill0 = jnp.where(in0, MASKED, -jnp.inf).astype(F32)
        fill1 = jnp.where(in1, MASKED, -jnp.inf).astype(F32)
        first_head = lane < Dh - LANES

        def block_diag(t):
            z = jnp.zeros((L, LANES), F32)
            mid = t[:, LANES:2 * LANES]
            top = jnp.concatenate([t[:, :LANES], jnp.where(first_head, mid, 0.0), z], axis=1)
            bot = jnp.concatenate([z, jnp.where(first_head, 0.0, mid), t[:, 2 * LANES:]], axis=1)
            pad = jnp.zeros((LANES - 2 * L, PW), F32)
            return jnp.concatenate([top, bot, pad], axis=0).astype(BF16)

        def pair_softmax(s):
            s = s * (b_scale * LOG2E)
            s0 = jnp.where(visible & in0, s, fill0)
            s1 = jnp.where(visible & in1, s, fill1)
            m0 = jnp.max(s0, axis=1, keepdims=True)
            m1 = jnp.max(s1, axis=1, keepdims=True)
            e = jnp.exp2(jnp.where(in0, s0 - m0, s1 - m1))
            d0 = jnp.sum(jnp.where(in0, e, 0.0), axis=1, keepdims=True)
            d1 = jnp.sum(jnp.where(in0, 0.0, e), axis=1, keepdims=True)
            return e / jnp.where(in0, d0, d1)

        def weight(t, p, k0=0, k1=D):
            return _unpack(w_p[1 + t * n_pair + p, k0 // 2:k1 // 2])

        def out_proj(p0, p1, r0=0):
            return _dot(o_s[r0:, p0 * PW:p1 * PW], wob_v[p0 * PW:p1 * PW, :])

        def attend(s):
            h_s[M:, :] = xb_v[_block(s, seg), :].astype(F32)
            prob = vbd = acc = None
            for p in range(n_pair):
                h = h_s[...]
                if p == 0:
                    c0 = D - LANES
                    k = _dot(h[:, c0:], weight(0, p, c0))
                    q = _dot(h[:, c0:], weight(1, p, c0))
                    k = k + _dot(h[:, :c0], weight(0, p, 0, c0))
                    q = q + _dot(h[:, :c0], weight(1, p, 0, c0))
                else:
                    k = _dot(h, weight(0, p))
                    q = _dot(h, weight(1, p))
                v = _dot(h, weight(2, p))
                if p > 0:
                    o_s[:, (p - 1) * PW:p * PW] = _dot(prob, vbd)
                if p == n_pair - 1:
                    acc = out_proj(0, 1)
                prob = pair_softmax(_dot_nt(q, block_diag(k)))
                vbd = block_diag(v)
            acc_s[...] = acc + out_proj(1, B_HEAD_PAIRS)
            o_s[:, (n_pair - 1) * PW:] = _dot(prob, vbd)

        def finish(s, last=False):
            if last:
                y = acc_s[M:, :] + out_proj(B_HEAD_PAIRS, n_pair, M)
            else:
                acc = acc_s[...] + out_proj(B_HEAD_PAIRS, n_pair)
                h_s[0:M, :] = acc[0:M]
                y = acc[M:]
            outb_v[_block(s, seg), :] = y.astype(BF16)
            outb_copy(_block(s, seg)).start()

        for cp in (mem_copy, xb_head, wo_head):
            cp.wait()
        h_s[0:M, :] = mem0_v[...].astype(F32)
        attend(0)
        wo_rest.wait()
        outa_copy.start()

        def b_step(i, carry):
            @pl.when(i == 1)
            def _():
                xb_rest.wait()

            for u in range(B_UNROLL):
                finish(i * B_UNROLL + u)
                attend(i * B_UNROLL + u + 1)
            return carry

        lax.fori_loop(0, (n_seg - 1) // B_UNROLL, b_step, 0)
        finish(n_seg - 1, last=True)

        outa_copy.wait()
        outb_copy(pl.ds(0, S)).wait()

    n_slot = 1 + 3 * n_pair
    scratch = [
        pltpu.VMEM((S, D), BF16),
        pltpu.VMEM((3, D, D), BF16),
        pltpu.VMEM((D, D), BF16),
        pltpu.VMEM((S, D), BF16),
        pltpu.VMEM((M, D), BF16),
        pltpu.VMEM((n_slot * PW, D), BF16),
        pltpu.VMEM((H * Dh, D), BF16),
        pltpu.VMEM((n_tile, D // 2, LANES), jnp.int32),
        pltpu.VMEM((4, D // 2, D), jnp.int32),
        pltpu.VMEM((A_CHUNK, D), F32),
        pltpu.VMEM((n_tile, A_HALO + A_CHUNK, LANES), F32),
        pltpu.VMEM((n_tile, A_HALO + A_CHUNK, LANES), F32),
        pltpu.VMEM((A_CHUNK, D), F32),
        pltpu.VMEM((S, D), BF16),
        pltpu.VMEM((n_slot, D // 2, PW), jnp.int32),
        pltpu.VMEM((L, D), F32),
        pltpu.VMEM((L, H * Dh), F32),
        pltpu.VMEM((L, D), F32),
        pltpu.VMEM((S, D), BF16),
        pltpu.SemaphoreType.DMA((SEM_W + n_chunk,)),
        pltpu.SemaphoreType.DMA((2,)),
    ]
    return kernel, scratch


@functools.partial(jax.jit, static_argnames=("B_seg_len",))
def pallas_concat_heads__sliding_local_dilated__memory_aug_recurrent_mem_tr__prompt_kernel(
    A_x, A_wqkv, A_wo, B_x, B_mem0, B_Wq, B_Wk, B_Wv, B_Wo, B_seg_len,
):
    _, S, D = A_x.shape
    _, H, Dh = B_Wq.shape
    M = B_mem0.shape[1]
    kernel, scratch = _make_kernel(S, D, H, Dh, M, B_seg_len)

    def features_first(w):
        return jnp.transpose(w, (1, 2, 0)).reshape(H * Dh, D)

    out = pl.pallas_call(
        kernel,
        out_shape=jax.ShapeDtypeStruct((S, 2 * D), BF16),
        in_specs=[pl.BlockSpec(memory_space=pl.ANY)] * 9,
        out_specs=pl.BlockSpec(memory_space=pl.ANY),
        scratch_shapes=scratch,
        compiler_params=pltpu.CompilerParams(vmem_limit_bytes=100 * 2**20),
    )(
        A_x.reshape(S, D), A_wqkv, A_wo, B_x.reshape(S, D), B_mem0.reshape(M, D),
        features_first(B_Wq), features_first(B_Wk), features_first(B_Wv), B_Wo.reshape(H * Dh, D),
    )
    return out.reshape(1, S, 2 * D)
```
